```python
import jax
import jax.numpy as jnp

def _softmax(x, axis=-1):
    return jax.nn.softmax(x, axis=axis)
def _gelu(x):
    return jax.nn.gelu(x, approximate=True)
def _silu(x):
    return jax.nn.silu(x)
def _sigmoid(x):
    return jax.nn.sigmoid(x)
def _layernorm(x, axis=-1, eps=1e-5):
    m = jnp.mean(x, axis=axis, keepdims=True)
    v = jnp.var(x, axis=axis, keepdims=True)
    return (x - m) / jnp.sqrt(v + eps)
def _scatter_add(tgt, idx, src, axis=0):
    return tgt.at[idx].add(src)
def _segment_sum(src, seg, n):
    return jax.ops.segment_sum(src, seg, n)
class _Rng:
    def __init__(self, key):
        self._k = key
    def _next(self):
        self._k, sub = jax.random.split(self._k)
        return sub
    def normal(self, shape):
        return jax.random.normal(self._next(), shape, dtype=jnp.bfloat16)
    def randint(self, lo, hi, shape):
        return jax.random.randint(self._next(), shape, lo, hi, dtype=jnp.int32)
    def uniform(self, shape, lo=0.0, hi=1.0):
        return jax.random.uniform(self._next(), shape, jnp.bfloat16, lo, hi)
    def permutation(self, n):
        return jax.random.permutation(self._next(), n)


kernel_name = 'interleave_layers__sliding_block_cached__mixer_s_mlp__decode'

def setup_inputs():
    _rng = _Rng(jax.random.key(int.from_bytes(__import__("os").urandom(4), "little")))
    _w = (lambda a: (lambda t: t.astype(jnp.bfloat16) if jnp.issubdtype(t.dtype, jnp.floating) else t)(jnp.asarray(a)))
    def _A_setup():
        B, Sq, D = 1, 1, 640
        Hq, Hkv, Sk, Dh = 32, 32, 32768, 192
        assert Hq % Hkv == 0, (Hq, Hkv)
        return {
            "x": _w((lambda *s: _rng.normal(s) * 0.05)(B, Sq, D)),
            "k_cache": _w((lambda *s: _rng.normal(s) * 0.05)(B, Hkv, Sk, Dh)),
            "v_cache": _w((lambda *s: _rng.normal(s) * 0.05)(B, Hkv, Sk, Dh)),
            "wq": _w((lambda *s: _rng.normal(s) * 0.05)(D, Hq * Dh) * (D ** -0.5)),
            "wo": _w((lambda *s: _rng.normal(s) * 0.05)(Hq * Dh, D) * ((Hq * Dh) ** -0.5)),
        }
    _A_in = _A_setup()

    def _B_setup():
        B, S, D, F = 1, 1, 640, 1536
        return {
            "x":  _w((lambda *s: _rng.normal(s) * 0.05)(B, S, D)),
            "w1": _w((lambda *s: _rng.normal(s) * 0.05)(D, D) * (D ** -0.5)),
            "w2": _w((lambda *s: _rng.normal(s) * 0.05)(D, D) * (D ** -0.5)),
            "w3": _w((lambda *s: _rng.normal(s) * 0.05)(D, F) * (D ** -0.5)),
            "w4": _w((lambda *s: _rng.normal(s) * 0.05)(F, D) * (F ** -0.5)),
        }
    _B_in = _B_setup()

    return {
        "A_x": _A_in["x"],
        "A_k_cache": _A_in["k_cache"],
        "A_v_cache": _A_in["v_cache"],
        "A_wq": _A_in["wq"],
        "A_wo": _A_in["wo"],
        "B_x": _B_in["x"],
        "B_w1": _B_in["w1"],
        "B_w2": _B_in["w2"],
        "B_w3": _B_in["w3"],
        "B_w4": _B_in["w4"],
    }

def reference(A_x, A_k_cache, A_v_cache, A_wq, A_wo, B_x, B_w1, B_w2, B_w3, B_w4):
    def _A_ref(x, k_cache, v_cache, wq, wo):
        B, Sq, D = x.shape
        Hq, Dh = 32, 192
        Hkv, Sk = k_cache.shape[1], k_cache.shape[2]
        W = min(4096, max(256, Sk // 4))
        rep = Hq // Hkv
        q = (lambda x, *d: x.transpose(*d))((x @ wq).reshape(B, Sq, Hq, Dh), 0, 2, 1, 3)
        k = jnp.repeat(k_cache[:, :, Sk - W:, :], rep, axis=1)
        v = jnp.repeat(v_cache[:, :, Sk - W:, :], rep, axis=1)
        scores = jnp.einsum("bhqd,bhkd->bhqk", q, k) * (Dh ** -0.5)
        p = _softmax(scores, axis=-1)
        o = jnp.einsum("bhqk,bhkd->bhqd", p, v)
        return (lambda x, *d: x.transpose(*d))(o, 0, 2, 1, 3).reshape(B, Sq, Hq * Dh) @ wo

    def _B_ref(x, w1, w2, w3, w4):
        B, S, D = x.shape
        h = _gelu(_layernorm(x, axis=-1) @ w1)
        c = D // 4
        g0 = jnp.pad(h[:, :, 0*c:1*c], ((0, 0), (1, 0), (0, 0)))[:, :S, :]
        g1 = jnp.pad(h[:, :, 1*c:2*c], ((0, 0), (0, 1), (0, 0)))[:, 1:, :]
        g2 = jnp.pad(h[:, :, 2*c:3*c], ((0, 0), (2, 0), (0, 0)))[:, :S, :]
        g3 = jnp.pad(h[:, :, 3*c:   ], ((0, 0), (0, 2), (0, 0)))[:, 2:, :]
        hs = jnp.concatenate([g0, g1, g2, g3], axis=-1) @ w2
        x1 = x + hs
        h2 = _gelu(_layernorm(x1, axis=-1) @ w3) @ w4
        return x1 + h2

    x = A_x
    x = x + _A_ref(_layernorm(x, axis=-1), A_k_cache, A_v_cache, A_wq, A_wo)
    x = x + _B_ref(_layernorm(x, axis=-1), B_w1, B_w2, B_w3, B_w4)
    x = x + _A_ref(_layernorm(x, axis=-1), A_k_cache, A_v_cache, A_wq, A_wo)
    x = x + _B_ref(_layernorm(x, axis=-1), B_w1, B_w2, B_w3, B_w4)
    return x
```

```python
import functools

import jax
import jax.numpy as jnp
import jax.experimental.pallas as pl
import jax.experimental.pallas.tpu as pltpu
from jax import lax

_H = 32
_DH = 192
_W = 4096
_D = 640
_F = 1536
_EPS = 1e-5
_PAD = 128
_BF = jnp.bfloat16
_F32 = jnp.float32


def _layernorm(x):
    m = jnp.mean(x, axis=-1, keepdims=True)
    d = x - m
    v = jnp.mean(d * d, axis=-1, keepdims=True)
    return d / jnp.sqrt(v + _EPS)


def _gelu(x):
    c = 0.7978845608028654
    return 0.5 * x * (1.0 + jnp.tanh(c * (x + 0.044715 * (x * x * x))))


def _dot(a, b):
    return jnp.dot(a, b, preferred_element_type=_F32)


def _dot_t(a, b):
    return lax.dot_general(a, b, (((1,), (1,)), ((), ())), preferred_element_type=_F32)


def _kernel(x_ref, k_hbm, v_hbm, wq_hbm, wo_hbm, w3_hbm, w4_hbm, o_ref,
            kbuf, vbuf, wqbuf, wobuf, w3buf, w4buf, acc_ref, sem_kv, sem_w, *, sk):
    G1 = 2
    NS = _H // G1
    R1 = G1 * _DH
    G2 = 8
    scale = float(_DH) ** -0.5

    def k_copy(i):
        return pltpu.make_async_copy(
            k_hbm.at[pl.ds(i * R1, R1), pl.ds(sk - _W, _W)],
            kbuf.at[pl.ds(i * R1, R1), pl.ds(0, _W)], sem_kv.at[0, i])

    def v_copy(i):
        return pltpu.make_async_copy(
            v_hbm.at[pl.ds(i * R1, R1), pl.ds(sk - _W, _W)],
            vbuf.at[pl.ds(i * R1, R1), pl.ds(0, _W)], sem_kv.at[1, i])

    def wo_copy(i):
        return pltpu.make_async_copy(
            wo_hbm.at[pl.ds(i * R1, R1), :], wobuf.at[pl.ds(i * R1, R1), :], sem_kv.at[2, i])

    wq_copy = pltpu.make_async_copy(wq_hbm, wqbuf.at[:, pl.ds(0, _H * _DH)], sem_w.at[0])
    w3_copy = pltpu.make_async_copy(w3_hbm, w3buf.at[:, pl.ds(0, _F)], sem_w.at[1])
    w4_copy = pltpu.make_async_copy(w4_hbm, w4buf, sem_w.at[2])

    wq_copy.start()
    for i in range(NS):
        k_copy(i).start()
        v_copy(i).start()
        wo_copy(i).start()
    w3_copy.start()
    w4_copy.start()

    def attend(xn8, r, G):
        R = G * _DH
        rows = pl.ds(r, R)
        row = lax.broadcasted_iota(jnp.int32, (8, R), 0)
        col = lax.broadcasted_iota(jnp.int32, (8, R), 1)
        own = (col >= row * _DH) & (col < (row + 1) * _DH)
        q8 = _dot(xn8, wqbuf[:, rows])
        qbd = jnp.where(own, q8, 0.0).astype(_BF)
        s = _dot(qbd, kbuf[rows, 0:_W]) * scale
        m = jnp.max(s, axis=-1, keepdims=True)
        e = jnp.exp(s - m)
        p = (e / jnp.sum(e, axis=-1, keepdims=True)).astype(_BF)
        o = _dot_t(p, vbuf[rows, 0:_W])
        obd = jnp.where(own, o, 0.0).astype(_BF)
        return _dot(obd, wobuf[rows, :])

    def mlp_in(x):
        y = _layernorm(x)
        yn = jnp.broadcast_to(_layernorm(y), (8, _D)).astype(_BF)
        h = _gelu(_dot(yn, w3buf[:, 0:_F])).astype(_BF)
        return y, h

    def mlp_out(x, y, h):
        return x + (y + _dot(h, w4buf[...])[0:1])

    x = x_ref[...].astype(_F32)
    xn8 = jnp.broadcast_to(_layernorm(x), (8, _D)).astype(_BF)
    acc_ref[...] = jnp.zeros_like(acc_ref)
    wq_copy.wait()

    @pl.loop(0, NS)
    def _(i):
        k_copy(i).wait()
        v_copy(i).wait()
        wo_copy(i).wait()
        acc_ref[...] += attend(xn8, pl.multiple_of(i * R1, R1), G1)

    x = x + jnp.sum(acc_ref[...], axis=0, keepdims=True)
    w3_copy.wait()
    y, h = mlp_in(x)
    w4_copy.wait()
    x = mlp_out(x, y, h)

    xn8 = jnp.broadcast_to(_layernorm(x), (8, _D)).astype(_BF)
    acc_ref[...] = jnp.zeros_like(acc_ref)

    @pl.loop(0, _H // G2)
    def _(g):
        acc_ref[...] += attend(xn8, pl.multiple_of(g * G2 * _DH, G2 * _DH), G2)

    x = x + jnp.sum(acc_ref[...], axis=0, keepdims=True)
    y, h = mlp_in(x)
    x = mlp_out(x, y, h)
    o_ref[...] = x.astype(o_ref.dtype)


@jax.jit
def pallas_interleave_layers__sliding_block_cached__mixer_s_mlp__decode_kernel(
    A_x: jax.Array,
    A_k_cache: jax.Array,
    A_v_cache: jax.Array,
    A_wq: jax.Array,
    A_wo: jax.Array,
    B_x: jax.Array,
    B_w1: jax.Array,
    B_w2: jax.Array,
    B_w3: jax.Array,
    B_w4: jax.Array,
):
    del B_x, B_w1, B_w2
    _, hkv, sk, dh = A_k_cache.shape
    assert (hkv, dh) == (_H, _DH) and min(4096, max(256, sk // 4)) == _W
    kt = jnp.swapaxes(A_k_cache, 2, 3).reshape(_H * _DH, sk)
    vt = jnp.swapaxes(A_v_cache, 2, 3).reshape(_H * _DH, sk)
    any_spec = pl.BlockSpec(memory_space=pl.ANY)
    out = pl.pallas_call(
        functools.partial(_kernel, sk=sk),
        out_shape=jax.ShapeDtypeStruct((1, _D), A_x.dtype),
        in_specs=[pl.BlockSpec(memory_space=pltpu.VMEM)] + [any_spec] * 6,
        out_specs=pl.BlockSpec(memory_space=pltpu.VMEM),
        scratch_shapes=[
            pltpu.VMEM((_H * _DH, _W + _PAD), _BF),
            pltpu.VMEM((_H * _DH, _W + _PAD), _BF),
            pltpu.VMEM((_D, _H * _DH + _PAD), _BF),
            pltpu.VMEM((_H * _DH, _D), _BF),
            pltpu.VMEM((_D, _F + _PAD), _BF),
            pltpu.VMEM((_F, _D), _BF),
            pltpu.VMEM((8, _D), _F32),
            pltpu.SemaphoreType.DMA((3, _H // 2)),
            pltpu.SemaphoreType.DMA((3,)),
        ],
        compiler_params=pltpu.CompilerParams(vmem_limit_bytes=127 * 1024 * 1024),
        name="interleave_decode",
    )(A_x.reshape(1, _D), kt, vt, A_wq, A_wo, B_w3, B_w4)
    return out.reshape(1, 1, _D)
```

```python
import functools

import jax
import jax.numpy as jnp
import jax.experimental.pallas as pl
import jax.experimental.pallas.tpu as pltpu
from jax import lax

_H = 32
_DH = 192
_W = 4096
_D = 640
_F = 1536
_EPS = 1e-5
_PAD = 128
_BF = jnp.bfloat16
_F32 = jnp.float32
_U32 = jnp.uint32

_NP = _H // 2
_R = 2 * _DH
_CK = 512
_RV = 32
_NX = 2
_SLK = 150
_PVC = 1.55
_SMC = 80
_NLAND = 2
_VAHEAD = 2
_WU32 = True


def _layernorm(x):
    m = jnp.mean(x, axis=-1, keepdims=True)
    d = x - m
    v = jnp.mean(d * d, axis=-1, keepdims=True)
    return d / jnp.sqrt(v + _EPS)


def _gelu(x):
    c = 0.7978845608028654
    return 0.5 * x * (1.0 + jnp.tanh(c * (x + 0.044715 * (x * x * x))))


def _dot(a, b):
    return jnp.dot(a, b, preferred_element_type=_F32)


def _dot_t(a, b):
    return lax.dot_general(a, b, (((1,), (1,)), ((), ())), preferred_element_type=_F32)


def _pair_masks():
    row = lax.broadcasted_iota(jnp.int32, (8, _R), 0)
    col = lax.broadcasted_iota(jnp.int32, (8, _R), 1)
    own = (col >= row * _DH) & (col < (row + 1) * _DH)
    return own, col < _DH


_C2 = float(_DH) ** -0.5 * 1.4426950408889634


def _softmax_parts(s, first):
    m = jnp.max(s, axis=-1, keepdims=True)
    e = jnp.exp2(s - m)
    inv = 1.0 / jnp.sum(e, axis=-1, keepdims=True)
    return e, jnp.where(first, inv[0:1, :], inv[1:2, :])


def _layer2(xn8, always, kres, vres, wq_of, wo_of):
    own, first = _pair_masks()
    sub = lax.broadcasted_iota(jnp.int32, (8, 128), 0)
    lane = lax.broadcasted_iota(jnp.int32, (8, 128), 1)

    def tie(a, b):
        return jnp.where(always, a, b)

    st = {}
    acc = [jnp.zeros((8, _D), _F32)]

    def q_unit(i):
        q8 = _dot(xn8, wq_of(i))
        st[i] = {"q": jnp.where(own, q8 * _C2, 0.0).astype(_BF), "s": [], "red": []}
        return q8[:, 0:128]

    def qk_unit(i, c):
        k = pltpu.bitcast(kres[i * _DH:(i + 1) * _DH, c * _CK:(c + 1) * _CK], _BF)
        s = _dot(st[i]["q"], k)
        st[i]["s"].append(s)
        return s[:, 0:128]

    def softmax(i):
        e, st[i]["inv"] = _softmax_parts(jnp.concatenate(st[i].pop("s"), axis=1), first)
        return e

    def pv_unit(i, hh, c, ties):
        r = i * _R + hh * _DH + c * _RV
        a = None
        for t in ties:
            a = tie(jnp.zeros((8, 128), _F32) if a is None else a, t)
        if a is not None:
            a = jnp.tile(a, (_RV // 8, 1))
        for j in range(_W // 128):
            p = jnp.tile(st[i]["p"][hh][j], (_RV // 8, 1))
            t = vres[r:r + _RV, j * 128:(j + 1) * 128].astype(_F32) * p
            a = t if a is None else a + t
        red = jnp.broadcast_to(jnp.sum(a, axis=1, keepdims=True), (_RV, 128))
        st[i]["red"].extend(red[8 * b:8 * b + 8] for b in range(_RV // 8))

    def o_unit(i):
        red = st[i].pop("red")
        tiles = []
        for t in range(_R // 128):
            lvl = red[16 * t:16 * t + 16]
            w = 8
            while len(lvl) > 1:
                lo = (lane & w) == 0
                lvl = [jnp.where(lo, lvl[2 * n], lvl[2 * n + 1]) for n in range(len(lvl) // 2)]
                w *= 2
            tiles.append(jnp.where((lane & 7) == sub, lvl[0], 0.0))
        lhs = (jnp.concatenate(tiles, axis=1) * st[i]["inv"]).astype(_BF)
        r = _dot(lhs, wo_of(i))
        acc[0] = acc[0] + r
        return r[:, 0:128]

    def px_unit(i, c):
        if c == 0:
            st[i]["e"] = softmax(i).astype(_BF)
        cols = slice(c * _CK, (c + 1) * _CK)
        o = _dot_t(st[i]["e"][:, cols], vres[i * _R:(i + 1) * _R, cols])
        st[i]["o"] = o if c == 0 else st[i]["o"] + o
        return o[:, 0:128]

    def ox_unit(i):
        lhs = (jnp.where(own, st[i].pop("o"), 0.0) * st[i]["inv"]).astype(_BF)
        r = _dot(lhs, wo_of(i))
        acc[0] = acc[0] + r
        return r[:, 0:128]

    nck = _W // _CK
    nrv = _DH // _RV
    t_w, t_qk, t_lat = 125, _R * _CK / 2048 * 1.03, 110
    t_pv = _RV * _W / 2048 * _PVC
    clock = {"m": 0.0, "v": 0.0}
    s_ready = {}
    pending = []
    mxu = [("q", 0, 0)]
    for i in range(_NP):
        if i + 1 < _NP:
            mxu.append(("q", i + 1, 0))
        mxu.extend(("qk", i, c) for c in range(nck))
    nv = _NP - _NX
    for i in range(nv, _NP):
        mxu.extend(("px", i, c) for c in range(nck))
    mxu.extend(("ox", i, 0) for i in range(nv, _NP))
    mxu.reverse()
    vpu = [(i, hh, c) for i in range(nv) for hh in range(2) for c in range(nrv)]
    vpu.reverse()
    o_queue = []

    def run_mxu():
        kind, i, c = mxu.pop()
        if kind == "q":
            v = q_unit(i)
            clock["m"] += t_w
        elif kind == "qk":
            v = qk_unit(i, c)
            clock["m"] += t_qk
            if c == nck - 1:
                s_ready[i] = clock["m"] + t_lat
        elif kind == "px":
            v = px_unit(i, c)
            clock["m"] += 2 * t_qk
        else:
            v = ox_unit(i)
            clock["m"] += t_w
        pending.append((clock["m"] + _SLK, v))

    def run_o():
        i, tv = o_queue.pop(0)
        clock["m"] = max(clock["m"], tv) + t_w
        pending.append((clock["m"] + _SLK, o_unit(i)))

    while vpu:
        i, hh, c = vpu.pop()
        if "p" not in st.get(i, ()):
            while i not in s_ready:
                run_mxu()
            e = softmax(i)
            st[i]["p"] = [[jnp.broadcast_to(e[h2:h2 + 1, j * 128:(j + 1) * 128], (8, 128))
                           for j in range(_W // 128)] for h2 in range(2)]
            clock["v"] = max(clock["v"], s_ready[i]) + _SMC
        while True:
            if o_queue and o_queue[0][1] <= clock["m"] + t_w:
                run_o()
            elif mxu and clock["m"] <= clock["v"] + t_pv:
                run_mxu()
            else:
                break
        ties = [v for (t, v) in pending if t <= clock["v"]]
        pending[:] = [(t, v) for (t, v) in pending if t > clock["v"]]
        pv_unit(i, hh, c, ties)
        clock["v"] += t_pv
        if hh == 1 and c == nrv - 1:
            del st[i]["p"]
            o_queue.append((i, clock["v"] + t_lat))
    while mxu:
        run_mxu()
    while o_queue:
        run_o()
    return jnp.sum(acc[0], axis=0, keepdims=True)


def _kernel(flag_ref, x_ref, k_hbm, v_hbm, wq_hbm, wo_hbm, w3_hbm, w4_hbm, o_ref,
            kland, kres, vres, wqland, wqres, woland, wores, w3buf, w4buf, acc_ref,
            sem_k, sem_v, sem_q, sem_o, sem_w, *, sk):
    def k_copy(i):
        return pltpu.make_async_copy(
            k_hbm.at[pl.ds(i * _R, _R), pl.ds(sk - _W, _W)],
            kland.at[i % _NLAND], sem_k.at[i % _NLAND])

    def v_copy(i):
        return pltpu.make_async_copy(
            v_hbm.at[pl.ds(i * _R, _R), pl.ds(sk - _W, _W)],
            vres.at[pl.ds(i * _R, _R), :], sem_v.at[i])

    if _WU32:
        def wq_copy(i):
            return pltpu.make_async_copy(
                wq_hbm.at[:, pl.ds(i * _R, _R)], wqland.at[i % 2], sem_q.at[i % 2])

        def wo_copy(i):
            return pltpu.make_async_copy(
                wo_hbm.at[pl.ds(i * _R, _R), :], woland.at[i % 2], sem_o.at[i % 2])

        def wq_of(i):
            return pltpu.bitcast(wqres[:, i * _R:(i + 1) * _R], _BF)

        def wo_of(i):
            return pltpu.bitcast(wores[i * _DH:(i + 1) * _DH, :], _BF)
    else:
        def wq_copy(i):
            return pltpu.make_async_copy(
                wq_hbm.at[:, pl.ds(i * _R, _R)], wqres.at[:, pl.ds(i * _R, _R)], sem_q.at[i])

        def wo_copy(i):
            return pltpu.make_async_copy(
                wo_hbm.at[pl.ds(i * _R, _R), :], wores.at[pl.ds(i * _R, _R), :], sem_o.at[i])

        def wq_of(i):
            return wqres[:, i * _R:(i + 1) * _R]

        def wo_of(i):
            return wores[i * _R:(i + 1) * _R, :]

    w3_copy = pltpu.make_async_copy(w3_hbm, w3buf.at[:, pl.ds(0, _F)], sem_w.at[0])
    w4_copy = pltpu.make_async_copy(w4_hbm, w4buf, sem_w.at[1])

    def start_pair(i):
        wq_copy(i).start()
        k_copy(i).start()
        wo_copy(i).start()

    for i in range(_NLAND):
        start_pair(i)
        if i < _VAHEAD:
            v_copy(i).start()

    own, first = _pair_masks()

    def mlp_in(x):
        y = _layernorm(x)
        yn = jnp.broadcast_to(_layernorm(y), (8, _D)).astype(_BF)
        h = _gelu(_dot(yn, w3buf[:, 0:_F])).astype(_BF)
        return y, h

    def mlp_out(x, y, h):
        return x + (y + _dot(h, w4buf[...])[0:1])

    x = x_ref[...].astype(_F32)
    xn8 = jnp.broadcast_to(_layernorm(x), (8, _D)).astype(_BF)
    acc_ref[...] = jnp.zeros_like(acc_ref)

    @pl.loop(0, _NP)
    def _(i):
        wq_copy(i).wait()
        k_copy(i).wait()
        wo_copy(i).wait()
        v_copy(i).wait()

        @pl.when(i + _VAHEAD < _NP)
        def _():
            v_copy(i + _VAHEAD).start()

        rk = pl.multiple_of(i * _DH, _DH)
        rv = pl.multiple_of(i * _R, _R)
        if _WU32:
            wq = wqland[i % 2]
            wo = woland[i % 2]
            wqres[:, pl.ds(rv, _R)] = pltpu.bitcast(wq, _U32)
            wores[pl.ds(rk, _DH), :] = pltpu.bitcast(wo, _U32)
        else:
            wq = wqres[:, pl.ds(rv, _R)]
            wo = wores[pl.ds(rv, _R), :]
        q = jnp.where(own, _dot(xn8, wq) * _C2, 0.0).astype(_BF)
        k = kland[i % _NLAND]
        kres[pl.ds(rk, _DH), :] = pltpu.bitcast(k, _U32)
        e, inv = _softmax_parts(_dot(q, k), first)
        o = _dot_t(e.astype(_BF), vres[pl.ds(rv, _R), :])
        lhs = (jnp.where(own, o, 0.0) * inv).astype(_BF)
        acc_ref[...] += _dot(lhs, wo)

        @pl.when(i + _NLAND < _NP)
        def _():
            start_pair(i + _NLAND)

        @pl.when(i + _NLAND == _NP)
        def _():
            w3_copy.start()
            w4_copy.start()

    x = x + jnp.sum(acc_ref[...], axis=0, keepdims=True)
    w3_copy.wait()
    y, h = mlp_in(x)
    w4_copy.wait()
    x = mlp_out(x, y, h)

    xn8 = jnp.broadcast_to(_layernorm(x), (8, _D)).astype(_BF)
    x = x + _layer2(xn8, flag_ref[0] == 0, kres, vres, wq_of, wo_of)
    y, h = mlp_in(x)
    x = mlp_out(x, y, h)
    o_ref[...] = x.astype(o_ref.dtype)


@jax.jit
def pallas_interleave_layers__sliding_block_cached__mixer_s_mlp__decode_kernel(
    A_x: jax.Array,
    A_k_cache: jax.Array,
    A_v_cache: jax.Array,
    A_wq: jax.Array,
    A_wo: jax.Array,
    B_x: jax.Array,
    B_w1: jax.Array,
    B_w2: jax.Array,
    B_w3: jax.Array,
    B_w4: jax.Array,
):
    del B_x, B_w1, B_w2
    _, hkv, sk, dh = A_k_cache.shape
    assert (hkv, dh) == (_H, _DH) and min(4096, max(256, sk // 4)) == _W
    kt = jnp.swapaxes(A_k_cache, 2, 3).reshape(_H * _DH, sk)
    vt = jnp.swapaxes(A_v_cache, 2, 3).reshape(_H * _DH, sk)
    any_spec = pl.BlockSpec(memory_space=pl.ANY)
    if _WU32:
        w_scratch = [
            pltpu.VMEM((2, _D, _R), _BF), pltpu.VMEM((_D // 2, _H * _DH), _U32),
            pltpu.VMEM((2, _R, _D), _BF), pltpu.VMEM((_H * _DH // 2, _D), _U32),
        ]
    else:
        w_scratch = [
            pltpu.VMEM((8, 128), _BF), pltpu.VMEM((_D, _H * _DH + _PAD), _BF),
            pltpu.VMEM((8, 128), _BF), pltpu.VMEM((_H * _DH, _D), _BF),
        ]
    out = pl.pallas_call(
        functools.partial(_kernel, sk=sk),
        out_shape=jax.ShapeDtypeStruct((1, _D), A_x.dtype),
        in_specs=[pl.BlockSpec(memory_space=pltpu.SMEM),
                  pl.BlockSpec(memory_space=pltpu.VMEM)] + [any_spec] * 6,
        out_specs=pl.BlockSpec(memory_space=pltpu.VMEM),
        scratch_shapes=[
            pltpu.VMEM((_NLAND, _R, _W), _BF),
            pltpu.VMEM((_H * _DH // 2, _W), _U32),
            pltpu.VMEM((_H * _DH, _W), _BF),
            *w_scratch,
            pltpu.VMEM((_D, _F + _PAD), _BF),
            pltpu.VMEM((_F, _D), _BF),
            pltpu.VMEM((8, _D), _F32),
            pltpu.SemaphoreType.DMA((_NLAND,)),
            pltpu.SemaphoreType.DMA((_NP,)),
            pltpu.SemaphoreType.DMA((_NP,)),
            pltpu.SemaphoreType.DMA((_NP,)),
            pltpu.SemaphoreType.DMA((2,)),
        ],
        compiler_params=pltpu.CompilerParams(vmem_limit_bytes=127 * 1024 * 1024),
        name="interleave_decode",
    )(jnp.zeros((1,), jnp.int32), A_x.reshape(1, _D), kt, vt, A_wq, A_wo, B_w3, B_w4)
    return out.reshape(1, 1, _D)
```

```python
import functools

import jax
import jax.numpy as jnp
import jax.experimental.pallas as pl
import jax.experimental.pallas.tpu as pltpu
from jax import lax

_H = 32
_DH = 192
_W = 4096
_D = 640
_F = 1536
_EPS = 1e-5
_PAD = 128
_BF = jnp.bfloat16
_F32 = jnp.float32
_U32 = jnp.uint32

_NP = _H // 2
_R = 2 * _DH
_CK = 512
_RV = 32
_NX = 2
_SLK = 100
_PVC = 1.55
_SMA = 250
_SMB = 800
_FLAGS = [None, {"XLA_TPU_FORCE_LP_LLO_SCHEDULER": True}, {"XLA_TPU_EVENLY_DISTRIBUTE_CRITICAL_NODES": True}, {"XLA_TPU_FORCE_LP_LLO_SCHEDULER": True, "XLA_TPU_EVENLY_DISTRIBUTE_CRITICAL_NODES": True}]
_FL = 0
_SLA = 1.2
_RDN = 300
_RX = 0
_CKX = 1024
_PXP = 0
_RDL = 600
_ORD = 0
_QS = 4
_TV0 = 0
_UN = 2
_SMC = 80
_NW4 = 3
_RXA = 128
_RXB = 256
_NLAND = 2
_VAHEAD = 2
_WU32 = True


def _layernorm(x):
    m = jnp.mean(x, axis=-1, keepdims=True)
    d = x - m
    v = jnp.mean(d * d, axis=-1, keepdims=True)
    return d / jnp.sqrt(v + _EPS)


def _gelu(x):
    c = 0.7978845608028654
    return 0.5 * x * (1.0 + jnp.tanh(c * (x + 0.044715 * (x * x * x))))


def _dot(a, b):
    return jnp.dot(a, b, preferred_element_type=_F32)


def _dot_t(a, b):
    return lax.dot_general(a, b, (((1,), (1,)), ((), ())), preferred_element_type=_F32)


def _pair_masks():
    row = lax.broadcasted_iota(jnp.int32, (8, _R), 0)
    col = lax.broadcasted_iota(jnp.int32, (8, _R), 1)
    own = (col >= row * _DH) & (col < (row + 1) * _DH)
    return own, col < _DH


_C2 = float(_DH) ** -0.5 * 1.4426950408889634


def _softmax_parts(s, first):
    m = jnp.max(s, axis=-1, keepdims=True)
    e = jnp.exp2(s - m)
    inv = 1.0 / jnp.sum(e, axis=-1, keepdims=True)
    return e, jnp.where(first, inv[0:1, :], inv[1:2, :])


def _layer2(xn8, always, kres, vres, wqres, wores, q_ref, s_ref, e_ref, inv_ref, lhs_ref, acc_ref):
    own, first = _pair_masks()
    sub = lax.broadcasted_iota(jnp.int32, (8, 128), 0)
    lane = lax.broadcasted_iota(jnp.int32, (8, 128), 1)

    def tie(a, b):
        return jnp.where(always, a, b)

    def rows(i, n):
        return pl.ds(i * n, n) if isinstance(i, int) else pl.ds(pl.multiple_of(i * n, n), n)

    def q_unit(i, slot):
        q8 = _dot(xn8, pltpu.bitcast(wqres[:, rows(i, _R)], _BF))
        q_ref[slot] = jnp.where(own, q8 * _C2, 0.0)
        return q8[:, 0:128]

    def qk_unit(i, slot, c):
        cols = slice(c * _CK, (c + 1) * _CK)
        s = _dot(q_ref[slot].astype(_BF), pltpu.bitcast(kres[rows(i, _DH), cols], _BF))
        s_ref[slot, :, cols] = s
        return s[:, 0:128]

    def o_unit(i, slot):
        r = _dot(lhs_ref[slot].astype(_BF), pltpu.bitcast(wores[rows(i, _DH), :], _BF))
        acc_ref[...] += r
        return r[:, 0:128]

    def softmax(slot):
        s = s_ref[slot]
        m = jnp.max(s, axis=-1, keepdims=True)
        e = jnp.exp2(s - m)
        inv = 1.0 / jnp.sum(e, axis=-1, keepdims=True)
        inv = jnp.where(first, inv[0:1, :], inv[1:2, :])
        e_ref[slot] = e
        inv_ref[slot] = inv
        return jnp.broadcast_to(m, (8, 128)), inv[:, 0:128]

    def pv_unit(i, slot, hh, c, ties, red):
        r0 = hh * _DH + c * _RV
        vrows = pl.ds(i * _R + r0, _RV) if isinstance(i, int) else pl.ds(pl.multiple_of(i * _R + r0, _RV), _RV)
        a = None
        for t in ties:
            a = tie(jnp.zeros((8, 128), _F32) if a is None else a, t)
        if a is not None:
            a = jnp.tile(a, (_RV // 8, 1))
        for j in range(_W // 128):
            p = jnp.broadcast_to(e_ref[slot, hh:hh + 1, j * 128:(j + 1) * 128], (8, 128))
            t = vres[vrows, j * 128:(j + 1) * 128].astype(_F32) * jnp.tile(p, (_RV // 8, 1))
            a = t if a is None else a + t
        a = jnp.broadcast_to(jnp.sum(a, axis=1, keepdims=True), (_RV, 128))
        for b in range(_RV // 8):
            v, w = a[8 * b:8 * b + 8], 8
            while red and red[-1][0] == w and w < 128:
                v = jnp.where((lane & w) == 0, red.pop()[1], v)
                w *= 2
            red.append((w, v))
        return red[-1][1]

    def px_unit(i, slot, c, ox, rx):
        cols = slice(c * _CKX, (c + 1) * _CKX)
        r0 = _R - rx
        vrows = pl.ds(i * _R + r0, rx) if isinstance(i, int) else pl.ds(pl.multiple_of(i * _R + r0, 32), rx)
        o = _dot_t(e_ref[slot, :, cols].astype(_BF), vres[vrows, cols])
        ox[0] = o if c == 0 else ox[0] + o
        return jnp.broadcast_to(o[:, 0:1], (8, 128))

    def lhs_unit(slot, red, ox, rx):
        parts = [jnp.where((lane & 7) == sub, v, 0.0)[:, 0:w] for (w, v) in red]
        if rx:
            parts.append(jnp.where(own[:, _R - rx:], ox[0], 0.0))
        lhs_ref[slot] = jnp.concatenate(parts, axis=1) * inv_ref[slot]

    nck = _W // _CK
    nrv = _DH // _RV
    t_w, t_qk = 125, _R * _CK / 2048 * 1.03
    t_pv = _RV * _W / 2048 * _PVC
    _UN_T = t_pv * (_R - _RX) / _RV
    t_px = _CKX / 2048 * 2.05

    def step(i, par, carry=(), rx=_RX, lo=0, hi=_NP):
        def ok(d):
            return (not isinstance(i, int)) or lo <= i + d < hi
        qk = [(t_qk, functools.partial(qk_unit, i + 2, par, c)) for c in range(nck)] if ok(2) else []
        qq = [(t_w, lambda: q_unit(i + 3, 1 - par))] if ok(3) else []
        oo = [(t_w, lambda: o_unit(i - 1, 1 - par))] if ok(-1) else []
        ox = [None]
        px = [(t_px * rx, functools.partial(px_unit, i, par, c, ox, rx)) for c in range(_W // _CKX)] if rx and ok(0) else []
        mxu = {0: qk + qq + oo, 1: oo + qq + qk, 2: qk + oo + qq, 3: qk[:_QS] + oo + qq + qk[_QS:]}[_ORD]
        if _PXP >= 100:
            out = []
            px0 = list(px)
            for n, u in enumerate(mxu):
                out.append(u)
                while px and (n + 1) * len(px0) >= (len(px0) - len(px) + 1) * len(mxu) if (px0 if px0 else False) else False:
                    out.append(px.pop(0))
            mxu = out + px
        else:
            mxu = mxu[:_PXP] + px + mxu[_PXP:]
        mxu.reverse()
        pending = [(t - _UN_T, v) for (t, v) in carry]
        if ok(1):
            m, inv = softmax(1 - par)
            pending += [(_SMA, m), (_SMB, inv)]
        if ok(0):
            tm, tv, red = 0.0, float(_TV0), []
            for hh in range(2):
                for c in range(max(0, min(_DH, _R - rx - hh * _DH)) // _RV):
                    while mxu and tm * _SLA + _SLK <= tv + 2 * t_pv + 200:
                        dt, f = mxu.pop()
                        tm += dt
                        pending.append((tm * _SLA + _SLK, f()))
                    ties = [v for (t, v) in pending if t <= tv]
                    pending = [(t, v) for (t, v) in pending if t > tv]
                    v = pv_unit(i, par, hh, c, ties, red)
                    tv += t_pv
                    pending.append((tv + _RDL, v))
        while mxu:
            mxu.pop()[1]()
        if ok(0):
            lhs_unit(par, red, ox, rx)
        return pending

    acc_ref[...] = jnp.zeros_like(acc_ref)
    carry = ()
    for i in range(-3, 1):
        carry = step(i, i % 2, carry)

    @pl.loop(0, (_NP - 4) // _UN)
    def _(n):
        carry = ()
        for u in range(1, _UN + 1):
            carry = step(_UN * n + u, u % 2, carry)

    carry = ()
    for i in range(_NP - 3, _NP + 1):
        carry = step(i, i % 2, carry, {_NP - 2: _RXA, _NP - 1: _RXB}.get(i, _RX))


def _kernel(flag_ref, x_hbm, k_hbm, v_hbm, wq_hbm, wo_hbm, w3_hbm, w4_hbm, o_ref,
            kland, kres, vres, wqland, wqres, woland, wores, w3buf, w4buf, acc_ref,
            q_ref, s_ref, e_ref, inv_ref, lhs_ref, x_ref, sem_k, sem_v, sem_q, sem_o, sem_w, *, sk):
    def k_copy(i):
        return pltpu.make_async_copy(
            k_hbm.at[pl.ds(i * _R, _R), pl.ds(sk - _W, _W)],
            kland.at[i % _NLAND], sem_k.at[i % _NLAND])

    def v_copy(i):
        return pltpu.make_async_copy(
            v_hbm.at[pl.ds(i * _R, _R), pl.ds(sk - _W, _W)],
            vres.at[pl.ds(i * _R, _R), :], sem_v.at[i % (_VAHEAD + 1)])

    if _WU32:
        def wq_copy(i):
            return pltpu.make_async_copy(
                wq_hbm.at[:, pl.ds(i * _R, _R)], wqland.at[i % 2], sem_q.at[i % 2])

        def wo_copy(i):
            return pltpu.make_async_copy(
                wo_hbm.at[pl.ds(i * _R, _R), :], woland.at[i % 2], sem_o.at[i % 2])

        def wq_of(i):
            return pltpu.bitcast(wqres[:, i * _R:(i + 1) * _R], _BF)

        def wo_of(i):
            return pltpu.bitcast(wores[i * _DH:(i + 1) * _DH, :], _BF)
    else:
        def wq_copy(i):
            return pltpu.make_async_copy(
                wq_hbm.at[:, pl.ds(i * _R, _R)], wqres.at[:, pl.ds(i * _R, _R)], sem_q.at[i])

        def wo_copy(i):
            return pltpu.make_async_copy(
                wo_hbm.at[pl.ds(i * _R, _R), :], wores.at[pl.ds(i * _R, _R), :], sem_o.at[i])

        def wq_of(i):
            return wqres[:, i * _R:(i + 1) * _R]

        def wo_of(i):
            return wores[i * _R:(i + 1) * _R, :]

    w3_copy = pltpu.make_async_copy(w3_hbm, w3buf.at[:, pl.ds(0, _F)], sem_w.at[0])
    fc = _F // _NW4
    w4_copies = [pltpu.make_async_copy(w4_hbm.at[pl.ds(n * fc, fc), :], w4buf.at[pl.ds(n * fc, fc), :], sem_w.at[1 + n]) for n in range(_NW4)]
    x_copy = pltpu.make_async_copy(x_hbm, x_ref, sem_w.at[0])

    def start_pair(i):
        wq_copy(i).start()
        k_copy(i).start()
        wo_copy(i).start()

    for i in range(_NLAND):
        start_pair(i)
        if i < _VAHEAD:
            v_copy(i).start()
        if i == 0:
            x_copy.start()

    own, first = _pair_masks()

    def mlp_in(x):
        y = _layernorm(x)
        my = jnp.mean(y, axis=-1, keepdims=True)
        vy = jnp.mean(y * y, axis=-1, keepdims=True) - my * my
        yn = (y - my) / jnp.sqrt(vy + _EPS)
        yn = jnp.broadcast_to(yn, (8, _D)).astype(_BF)
        h = _gelu(_dot(yn, w3buf[:, 0:_F])).astype(_BF)
        return y, h

    def mlp_out(x, y, h, wait=False):
        out = x + y
        for n in range(_NW4):
            if wait:
                w4_copies[n].wait()
            out = out + _dot(h[:, n * fc:(n + 1) * fc], w4buf[n * fc:(n + 1) * fc, :])[0:1]
        return out

    x_copy.wait()
    x = x_ref[...].astype(_F32)
    xn8 = jnp.broadcast_to(_layernorm(x), (8, _D)).astype(_BF)
    acc_ref[...] = jnp.zeros_like(acc_ref)

    @pl.loop(0, _NP)
    def _(i):
        wq_copy(i).wait()
        k_copy(i).wait()
        wo_copy(i).wait()
        v_copy(i).wait()

        @pl.when(i + _VAHEAD < _NP)
        def _():
            v_copy(i + _VAHEAD).start()

        rk = pl.multiple_of(i * _DH, _DH)
        rv = pl.multiple_of(i * _R, _R)
        if _WU32:
            wq = wqland[i % 2]
            wo = woland[i % 2]
            wqres[:, pl.ds(rv, _R)] = pltpu.bitcast(wq, _U32)
            wores[pl.ds(rk, _DH), :] = pltpu.bitcast(wo, _U32)
        else:
            wq = wqres[:, pl.ds(rv, _R)]
            wo = wores[pl.ds(rv, _R), :]
        q = jnp.where(own, _dot(xn8, wq) * _C2, 0.0).astype(_BF)
        k = kland[i % _NLAND]
        kres[pl.ds(rk, _DH), :] = pltpu.bitcast(k, _U32)
        e, inv = _softmax_parts(_dot(q, k), first)
        o = _dot_t(e.astype(_BF), vres[pl.ds(rv, _R), :])
        lhs = (jnp.where(own, o, 0.0) * inv).astype(_BF)
        acc_ref[...] += _dot(lhs, wo)

        @pl.when(i + _NLAND < _NP)
        def _():
            start_pair(i + _NLAND)

        @pl.when(i + _NLAND == _NP)
        def _():
            w3_copy.start()
            for c in w4_copies:
                c.start()

    x = x + jnp.sum(acc_ref[...], axis=0, keepdims=True)
    w3_copy.wait()
    y, h = mlp_in(x)
    x = mlp_out(x, y, h, wait=True)

    xn8 = jnp.broadcast_to(_layernorm(x), (8, _D)).astype(_BF)
    _layer2(xn8, flag_ref[0] == 0, kres, vres, wqres, wores, q_ref, s_ref, e_ref, inv_ref, lhs_ref, acc_ref)
    x = x + jnp.sum(acc_ref[...], axis=0, keepdims=True)
    y, h = mlp_in(x)
    x = mlp_out(x, y, h)
    o_ref[...] = x.astype(o_ref.dtype)


@jax.jit
def pallas_interleave_layers__sliding_block_cached__mixer_s_mlp__decode_kernel(
    A_x: jax.Array,
    A_k_cache: jax.Array,
    A_v_cache: jax.Array,
    A_wq: jax.Array,
    A_wo: jax.Array,
    B_x: jax.Array,
    B_w1: jax.Array,
    B_w2: jax.Array,
    B_w3: jax.Array,
    B_w4: jax.Array,
):
    del B_x, B_w1, B_w2
    _, hkv, sk, dh = A_k_cache.shape
    assert (hkv, dh) == (_H, _DH) and min(4096, max(256, sk // 4)) == _W
    kt = jnp.swapaxes(A_k_cache, 2, 3).reshape(_H * _DH, sk)
    vt = jnp.swapaxes(A_v_cache, 2, 3).reshape(_H * _DH, sk)
    any_spec = pl.BlockSpec(memory_space=pl.ANY)
    if _WU32:
        w_scratch = [
            pltpu.VMEM((2, _D, _R), _BF), pltpu.VMEM((_D // 2, _H * _DH), _U32),
            pltpu.VMEM((2, _R, _D), _BF), pltpu.VMEM((_H * _DH // 2, _D), _U32),
        ]
    else:
        w_scratch = [
            pltpu.VMEM((8, 128), _BF), pltpu.VMEM((_D, _H * _DH + _PAD), _BF),
            pltpu.VMEM((8, 128), _BF), pltpu.VMEM((_H * _DH, _D), _BF),
        ]
    out = pl.pallas_call(
        functools.partial(_kernel, sk=sk),
        out_shape=jax.ShapeDtypeStruct((1, _D), A_x.dtype),
        in_specs=[pl.BlockSpec(memory_space=pltpu.SMEM),
                  any_spec] + [any_spec] * 6,
        out_specs=pl.BlockSpec(memory_space=pltpu.VMEM),
        scratch_shapes=[
            pltpu.VMEM((_NLAND, _R, _W), _BF),
            pltpu.VMEM((_H * _DH // 2, _W), _U32),
            pltpu.VMEM((_H * _DH, _W), _BF),
            *w_scratch,
            pltpu.VMEM((_D, _F + _PAD), _BF),
            pltpu.VMEM((_F, _D), _BF),
            pltpu.VMEM((8, _D), _F32),
            pltpu.VMEM((2, 8, _R), _F32),
            pltpu.VMEM((2, 8, _W), _F32),
            pltpu.VMEM((2, 8, _W), _F32),
            pltpu.VMEM((2, 8, _R), _F32),
            pltpu.VMEM((2, 8, _R), _F32),
            pltpu.VMEM((1, _D), _BF),
            pltpu.SemaphoreType.DMA((_NLAND,)),
            pltpu.SemaphoreType.DMA((_VAHEAD + 1,)),
            pltpu.SemaphoreType.DMA((2,)),
            pltpu.SemaphoreType.DMA((2,)),
            pltpu.SemaphoreType.DMA((1 + _NW4,)),
        ],
        compiler_params=pltpu.CompilerParams(vmem_limit_bytes=127 * 1024 * 1024, flags=_FLAGS[_FL]),
        name="interleave_decode",
    )(jnp.zeros((1,), jnp.int32), A_x.reshape(1, _D), kt, vt, A_wq, A_wo, B_w3, B_w4)
    return out.reshape(1, 1, _D)
```

```python
import functools

import jax
import jax.numpy as jnp
import jax.experimental.pallas as pl
import jax.experimental.pallas.tpu as pltpu
from jax import lax

_H = 32
_DH = 192
_W = 4096
_D = 640
_F = 1536
_EPS = 1e-5
_PAD = 128
_BF = jnp.bfloat16
_F32 = jnp.float32
_U32 = jnp.uint32

_NP = _H // 2
_R = 2 * _DH
_CK = 512
_RV = 32
_NX = 2
_SLK = 40
_PVC = 1.6
_SMA = 150
_SMB = 800
_FLAGS = [None, {"XLA_TPU_FORCE_LP_LLO_SCHEDULER": True}, {"XLA_TPU_EVENLY_DISTRIBUTE_CRITICAL_NODES": True}, {"XLA_TPU_FORCE_LP_LLO_SCHEDULER": True, "XLA_TPU_EVENLY_DISTRIBUTE_CRITICAL_NODES": True}]
_FL = 0
_SLA = 1.0
_RDN = 300
_RX = 0
_CKX = 1024
_PXP = 0
_RDL = 900
_ORD = 0
_QS = 4
_TV0 = 40
_UN = 2
_SMC = 80
_DALL = True
_NCH = 2
_NW4 = 3
_RXA = 192
_RXB = 192
_NLAND = 2
_VAHEAD = 2
_WU32 = True


def _layernorm(x):
    m = jnp.mean(x, axis=-1, keepdims=True)
    d = x - m
    v = jnp.mean(d * d, axis=-1, keepdims=True)
    return d / jnp.sqrt(v + _EPS)


def _gelu(x):
    c = 0.7978845608028654
    return 0.5 * x * (1.0 + jnp.tanh(c * (x + 0.044715 * (x * x * x))))


def _dot(a, b):
    return jnp.dot(a, b, preferred_element_type=_F32)


def _dot_t(a, b):
    return lax.dot_general(a, b, (((1,), (1,)), ((), ())), preferred_element_type=_F32)


def _pair_masks():
    row = lax.broadcasted_iota(jnp.int32, (8, _R), 0)
    col = lax.broadcasted_iota(jnp.int32, (8, _R), 1)
    own = (col >= row * _DH) & (col < (row + 1) * _DH)
    return own, col < _DH


_C2 = float(_DH) ** -0.5 * 1.4426950408889634


def _softmax_parts(s, first):
    m = jnp.max(s, axis=-1, keepdims=True)
    e = jnp.exp2(s - m)
    inv = 1.0 / jnp.sum(e, axis=-1, keepdims=True)
    return e, jnp.where(first, inv[0:1, :], inv[1:2, :])


def _layer2(xn8, always, kres, vres, wqres, wores, q_ref, s_ref, e_ref, inv_ref, lhs_ref, d_ref, acc_ref):
    own, first = _pair_masks()
    sub = lax.broadcasted_iota(jnp.int32, (8, 128), 0)
    lane = lax.broadcasted_iota(jnp.int32, (8, 128), 1)

    def tie(a, b):
        return jnp.where(always, a, b)

    def rows(i, n):
        return pl.ds(i * n, n) if isinstance(i, int) else pl.ds(pl.multiple_of(i * n, n), n)

    def q_unit(i, slot):
        q8 = _dot(xn8, pltpu.bitcast(wqres[:, rows(i, _R)], _BF))
        q_ref[slot] = jnp.where(own, q8 * _C2, 0.0)
        return q8[:, 0:128]

    def qk_unit(i, slot, c):
        cols = slice(c * _CK, (c + 1) * _CK)
        s = _dot(q_ref[slot].astype(_BF), pltpu.bitcast(kres[rows(i, _DH), cols], _BF))
        s_ref[slot, :, cols] = s
        return s[:, 0:128]

    def o_unit(i, lhs):
        r = _dot(lhs.astype(_BF), pltpu.bitcast(wores[rows(i, _DH), :], _BF))
        acc_ref[...] += r
        return r[:, 0:128]

    def softmax(slot):
        s = s_ref[slot]
        m = jnp.max(s, axis=-1, keepdims=True)
        e = jnp.exp2(s - m)
        inv = 1.0 / jnp.sum(e, axis=-1, keepdims=True)
        inv = jnp.where(first, inv[0:1, :], inv[1:2, :])
        e_ref[slot] = e
        inv_ref[slot] = inv
        return jnp.broadcast_to(m, (8, 128)), inv[:, 0:128]

    def fold_rows(a, red):
        a = jnp.broadcast_to(jnp.sum(a, axis=1, keepdims=True), a.shape)
        for b in range(a.shape[0] // 8):
            v, w = a[8 * b:8 * b + 8], 8
            while red and red[-1][0] == w and w < 128:
                v = jnp.where((lane & w) == 0, red.pop()[1], v)
                w *= 2
            red.append((w, v))
        return red[-1][1]

    def pv_unit(i, slot, hh, c, ties, red, defer=False):
        r0 = hh * _DH + c * _RV
        vrows = pl.ds(i * _R + r0, _RV) if isinstance(i, int) else pl.ds(pl.multiple_of(i * _R + r0, _RV), _RV)
        a = None
        for t in ties:
            a = tie(jnp.zeros((8, 128), _F32) if a is None else a, t)
        if a is not None:
            a = jnp.tile(a, (_RV // 8, 1))
        accs = [a] + [None] * (_NCH - 1)
        for j in range(_W // 128):
            p = jnp.broadcast_to(e_ref[slot, hh:hh + 1, j * 128:(j + 1) * 128], (8, 128))
            t = vres[vrows, j * 128:(j + 1) * 128].astype(_F32) * jnp.tile(p, (_RV // 8, 1))
            n = j % _NCH
            accs[n] = t if accs[n] is None else accs[n] + t
        a = accs[0]
        for t in accs[1:]:
            a = a + t
        if defer:
            d_ref[0:_RV, :] = a
            return a[0:8]
        return fold_rows(a, red)

    def px_unit(i, slot, c, ox, rx):
        cols = slice(c * _CKX, (c + 1) * _CKX)
        r0 = _R - rx
        vrows = pl.ds(i * _R + r0, rx) if isinstance(i, int) else pl.ds(pl.multiple_of(i * _R + r0, 32), rx)
        o = _dot_t(e_ref[slot, :, cols].astype(_BF), vres[vrows, cols])
        ox[0] = o if c == 0 else ox[0] + o
        return jnp.broadcast_to(o[:, 0:1], (8, 128))

    def make_lhs(slot, red, ox, rx):
        parts = [jnp.where((lane & 7) == sub, v, 0.0)[:, 0:w] for (w, v) in red]
        if rx:
            parts.append(jnp.where(own[:, _R - rx:], ox[0], 0.0))
        return jnp.concatenate(parts, axis=1) * inv_ref[slot]

    def park(red):
        for n, (_, v) in enumerate(red):
            d_ref[_RV + 8 * n:_RV + 8 * n + 8, :] = v

    def unpark(slot):
        widths = []
        for b in range((_R - _RV) // 8):
            w = 8
            while widths and widths[-1] == w and w < 128:
                widths.pop()
                w *= 2
            widths.append(w)
        red = [(w, d_ref[_RV + 8 * n:_RV + 8 * n + 8, :]) for n, w in enumerate(widths)]
        fold_rows(d_ref[0:_RV, :], red)
        return make_lhs(slot, red, None, 0)

    nck = _W // _CK
    nrv = _DH // _RV
    t_w, t_qk = 125, _R * _CK / 2048 * 1.03
    t_pv = _RV * _W / 2048 * _PVC
    _UN_T = t_pv * (_R - _RX) / _RV
    t_px = _CKX / 2048 * 2.05

    def step(i, par, carry=(), rx=_RX, defer=False, parked=False, lo=0, hi=_NP):
        def ok(d):
            return (not isinstance(i, int)) or lo <= i + d < hi
        qk = [(t_qk, functools.partial(qk_unit, i + 2, par, c)) for c in range(nck)] if ok(2) else []
        qq = [(t_w, lambda: q_unit(i + 3, 1 - par))] if ok(3) else []
        lhs = None if not ok(-1) else unpark(1 - par) if parked else None
        oo = [(t_w, lambda: o_unit(i - 1, lhs_ref[1 - par] if lhs is None else lhs))] if ok(-1) else []
        ox = [None]
        px = [(t_px * rx, functools.partial(px_unit, i, par, c, ox, rx)) for c in range(_W // _CKX)] if rx and ok(0) else []
        mxu = {0: qk + qq + oo, 1: oo + qq + qk, 2: qk + oo + qq, 3: qk[:_QS] + oo + qq + qk[_QS:]}[_ORD]
        if _PXP >= 100:
            out = []
            px0 = list(px)
            for n, u in enumerate(mxu):
                out.append(u)
                while px and (n + 1) * len(px0) >= (len(px0) - len(px) + 1) * len(mxu) if (px0 if px0 else False) else False:
                    out.append(px.pop(0))
            mxu = out + px
        else:
            mxu = mxu[:_PXP] + px + mxu[_PXP:]
        mxu.reverse()
        pending = [(t - _UN_T, v) for (t, v) in carry]
        if ok(1):
            m, inv = softmax(1 - par)
            pending += [(_SMA, m), (_SMB, inv)]
        if ok(0):
            tm, tv, red = 0.0, float(_TV0), []
            for hh in range(2):
                for c in range(max(0, min(_DH, _R - rx - hh * _DH)) // _RV):
                    while mxu and tm * _SLA + _SLK <= tv + 2 * t_pv + 200:
                        dt, f = mxu.pop()
                        tm += dt
                        pending.append((tm * _SLA + _SLK, f()))
                    ties = [v for (t, v) in pending if t <= tv]
                    pending = [(t, v) for (t, v) in pending if t > tv]
                    last = defer and hh == 1 and c == nrv - 1
                    v = pv_unit(i, par, hh, c, ties, red, last)
                    tv += t_pv
                    pending.append((tv + _RDL, v))
        while mxu:
            mxu.pop()[1]()
        if ok(0):
            if defer:
                park(red)
            else:
                lhs_ref[par] = make_lhs(par, red, ox, rx)
        return pending

    acc_ref[...] = jnp.zeros_like(acc_ref)
    carry = ()
    for i in range(-3, 1):
        carry = step(i, i % 2, carry, defer=i == 0)

    @pl.loop(0, (_NP - 4) // _UN)
    def _(n):
        carry = ()
        for u in range(1, _UN + 1):
            carry = step(_UN * n + u, u % 2, carry, _RX, defer=u == _UN or _DALL, parked=u == 1 or _DALL)

    carry = ()
    for i in range(_NP - 3, _NP + 1):
        carry = step(i, i % 2, carry, {_NP - 2: _RXA, _NP - 1: _RXB}.get(i, _RX), parked=i == _NP - 3)


def _kernel(x_hbm, k_hbm, v_hbm, wq_hbm, wo_hbm, w3_hbm, w4_hbm, o_ref,
            kland, kres, vres, wqland, wqres, woland, wores, w3buf, w4buf, acc_ref,
            q_ref, s_ref, e_ref, inv_ref, lhs_ref, d_ref, x_ref, sem_k, sem_v, sem_q, sem_o, sem_w, *, sk):
    def k_copy(i):
        return pltpu.make_async_copy(
            k_hbm.at[pl.ds(i * _R, _R), pl.ds(sk - _W, _W)],
            kland.at[i % _NLAND], sem_k.at[i % _NLAND])

    def v_copy(i):
        return pltpu.make_async_copy(
            v_hbm.at[pl.ds(i * _R, _R), pl.ds(sk - _W, _W)],
            vres.at[pl.ds(i * _R, _R), :], sem_v.at[i % (_VAHEAD + 1)])

    if _WU32:
        def wq_copy(i):
            return pltpu.make_async_copy(
                wq_hbm.at[:, pl.ds(i * _R, _R)], wqland.at[i % 2], sem_q.at[i % 2])

        def wo_copy(i):
            return pltpu.make_async_copy(
                wo_hbm.at[pl.ds(i * _R, _R), :], woland.at[i % 2], sem_o.at[i % 2])

        def wq_of(i):
            return pltpu.bitcast(wqres[:, i * _R:(i + 1) * _R], _BF)

        def wo_of(i):
            return pltpu.bitcast(wores[i * _DH:(i + 1) * _DH, :], _BF)
    else:
        def wq_copy(i):
            return pltpu.make_async_copy(
                wq_hbm.at[:, pl.ds(i * _R, _R)], wqres.at[:, pl.ds(i * _R, _R)], sem_q.at[i])

        def wo_copy(i):
            return pltpu.make_async_copy(
                wo_hbm.at[pl.ds(i * _R, _R), :], wores.at[pl.ds(i * _R, _R), :], sem_o.at[i])

        def wq_of(i):
            return wqres[:, i * _R:(i + 1) * _R]

        def wo_of(i):
            return wores[i * _R:(i + 1) * _R, :]

    w3_copy = pltpu.make_async_copy(w3_hbm, w3buf.at[:, pl.ds(0, _F)], sem_w.at[0])
    fc = _F // _NW4
    w4_copies = [pltpu.make_async_copy(w4_hbm.at[pl.ds(n * fc, fc), :], w4buf.at[pl.ds(n * fc, fc), :], sem_w.at[1 + n]) for n in range(_NW4)]
    x_copy = pltpu.make_async_copy(x_hbm, x_ref, sem_w.at[0])

    def start_pair(i):
        wq_copy(i).start()
        k_copy(i).start()
        wo_copy(i).start()

    for i in range(_NLAND):
        start_pair(i)
        if i < _VAHEAD:
            v_copy(i).start()
        if i == 0:
            x_copy.start()

    own, first = _pair_masks()

    def mlp_in(x):
        y = _layernorm(x)
        my = jnp.mean(y, axis=-1, keepdims=True)
        vy = jnp.mean(y * y, axis=-1, keepdims=True) - my * my
        yn = (y - my) / jnp.sqrt(vy + _EPS)
        yn = jnp.broadcast_to(yn, (8, _D)).astype(_BF)
        h = _gelu(_dot(yn, w3buf[:, 0:_F])).astype(_BF)
        return y, h

    def mlp_out(x, y, h, wait=False):
        out = x + y
        for n in range(_NW4):
            if wait:
                w4_copies[n].wait()
            out = out + _dot(h[:, n * fc:(n + 1) * fc], w4buf[n * fc:(n + 1) * fc, :])[0:1]
        return out

    x_copy.wait()
    x = x_ref[...].astype(_F32)
    always = ~(jnp.abs(jnp.broadcast_to(x[:, 0:128], (8, 128))) < 0.0)
    xn8 = jnp.broadcast_to(_layernorm(x), (8, _D)).astype(_BF)
    acc_ref[...] = jnp.zeros_like(acc_ref)

    @pl.loop(0, _NP)
    def _(i):
        wq_copy(i).wait()
        k_copy(i).wait()
        wo_copy(i).wait()
        v_copy(i).wait()

        @pl.when(i + _VAHEAD < _NP)
        def _():
            v_copy(i + _VAHEAD).start()

        rk = pl.multiple_of(i * _DH, _DH)
        rv = pl.multiple_of(i * _R, _R)
        if _WU32:
            wq = wqland[i % 2]
            wo = woland[i % 2]
            wqres[:, pl.ds(rv, _R)] = pltpu.bitcast(wq, _U32)
            wores[pl.ds(rk, _DH), :] = pltpu.bitcast(wo, _U32)
        else:
            wq = wqres[:, pl.ds(rv, _R)]
            wo = wores[pl.ds(rv, _R), :]
        q = jnp.where(own, _dot(xn8, wq) * _C2, 0.0).astype(_BF)
        k = kland[i % _NLAND]
        kres[pl.ds(rk, _DH), :] = pltpu.bitcast(k, _U32)
        e, inv = _softmax_parts(_dot(q, k), first)
        o = _dot_t(e.astype(_BF), vres[pl.ds(rv, _R), :])
        lhs = (jnp.where(own, o, 0.0) * inv).astype(_BF)
        acc_ref[...] += _dot(lhs, wo)

        @pl.when(i + _NLAND < _NP)
        def _():
            start_pair(i + _NLAND)

        @pl.when(i + _NLAND == _NP)
        def _():
            w3_copy.start()
            for c in w4_copies:
                c.start()

    x = x + jnp.sum(acc_ref[...], axis=0, keepdims=True)
    w3_copy.wait()
    y, h = mlp_in(x)
    x = mlp_out(x, y, h, wait=True)

    xn8 = jnp.broadcast_to(_layernorm(x), (8, _D)).astype(_BF)
    _layer2(xn8, always, kres, vres, wqres, wores, q_ref, s_ref, e_ref, inv_ref, lhs_ref, d_ref, acc_ref)
    x = x + jnp.sum(acc_ref[...], axis=0, keepdims=True)
    y, h = mlp_in(x)
    x = mlp_out(x, y, h)
    o_ref[...] = x.astype(o_ref.dtype)


@jax.jit
def pallas_interleave_layers__sliding_block_cached__mixer_s_mlp__decode_kernel(
    A_x: jax.Array,
    A_k_cache: jax.Array,
    A_v_cache: jax.Array,
    A_wq: jax.Array,
    A_wo: jax.Array,
    B_x: jax.Array,
    B_w1: jax.Array,
    B_w2: jax.Array,
    B_w3: jax.Array,
    B_w4: jax.Array,
):
    del B_x, B_w1, B_w2
    _, hkv, sk, dh = A_k_cache.shape
    assert (hkv, dh) == (_H, _DH) and min(4096, max(256, sk // 4)) == _W
    kt = jnp.swapaxes(A_k_cache, 2, 3).reshape(_H * _DH, sk)
    vt = jnp.swapaxes(A_v_cache, 2, 3).reshape(_H * _DH, sk)
    any_spec = pl.BlockSpec(memory_space=pl.ANY)
    if _WU32:
        w_scratch = [
            pltpu.VMEM((2, _D, _R), _BF), pltpu.VMEM((_D // 2, _H * _DH), _U32),
            pltpu.VMEM((2, _R, _D), _BF), pltpu.VMEM((_H * _DH // 2, _D), _U32),
        ]
    else:
        w_scratch = [
            pltpu.VMEM((8, 128), _BF), pltpu.VMEM((_D, _H * _DH + _PAD), _BF),
            pltpu.VMEM((8, 128), _BF), pltpu.VMEM((_H * _DH, _D), _BF),
        ]
    out = pl.pallas_call(
        functools.partial(_kernel, sk=sk),
        out_shape=jax.ShapeDtypeStruct((1, _D), A_x.dtype),
        in_specs=[any_spec] * 7,
        out_specs=pl.BlockSpec(memory_space=pltpu.VMEM),
        scratch_shapes=[
            pltpu.VMEM((_NLAND, _R, _W), _BF),
            pltpu.VMEM((_H * _DH // 2, _W), _U32),
            pltpu.VMEM((_H * _DH, _W), _BF),
            *w_scratch,
            pltpu.VMEM((_D, _F + _PAD), _BF),
            pltpu.VMEM((_F, _D), _BF),
            pltpu.VMEM((8, _D), _F32),
            pltpu.VMEM((2, 8, _R), _F32),
            pltpu.VMEM((2, 8, _W), _F32),
            pltpu.VMEM((2, 8, _W), _F32),
            pltpu.VMEM((2, 8, _R), _F32),
            pltpu.VMEM((2, 8, _R), _F32),
            pltpu.VMEM((_RV + 64, 128), _F32),
            pltpu.VMEM((1, _D), _BF),
            pltpu.SemaphoreType.DMA((_NLAND,)),
            pltpu.SemaphoreType.DMA((_VAHEAD + 1,)),
            pltpu.SemaphoreType.DMA((2,)),
            pltpu.SemaphoreType.DMA((2,)),
            pltpu.SemaphoreType.DMA((1 + _NW4,)),
        ],
        compiler_params=pltpu.CompilerParams(vmem_limit_bytes=127 * 1024 * 1024, flags=_FLAGS[_FL]),
        name="interleave_decode",
    )(A_x.reshape(1, _D), kt, vt, A_wq, A_wo, B_w3, B_w4)
    return out.reshape(1, 1, _D)
```

```python
import functools

import jax
import jax.numpy as jnp
import jax.experimental.pallas as pl
import jax.experimental.pallas.tpu as pltpu
from jax import lax

_H = 32
_DH = 192
_W = 4096
_D = 640
_F = 1536
_EPS = 1e-5
_PAD = 128
_BF = jnp.bfloat16
_F32 = jnp.float32
_U32 = jnp.uint32

_NP = _H // 2
_R = 2 * _DH
_CK = 512
_RV = 32
_NX = 2
_SLK = 40
_PVC = 1.6
_SMA = 150
_SMB = 900
_FLAGS = [None, {"XLA_TPU_FORCE_LP_LLO_SCHEDULER": True}, {"XLA_TPU_EVENLY_DISTRIBUTE_CRITICAL_NODES": True}, {"XLA_TPU_FORCE_LP_LLO_SCHEDULER": True, "XLA_TPU_EVENLY_DISTRIBUTE_CRITICAL_NODES": True}]
_FL = 0
_SLA = 1.0
_RDN = 300
_RX = 0
_CKX = 1024
_PXP = 0
_RDL = 900
_ORD = 0
_QS = 4
_TV0 = 40
_UN = 2
_SMC = 80
_DALL = True
_NCH = 2
_AH = (6,)
_A0 = 4
_A1 = 6
_SMP = 150
_SMQ = 450
_OPOS = 100
_NW4 = 3
_RXA = 192
_RXB = 192
_NLAND = 2
_VAHEAD = 2
_WU32 = True


def _layernorm(x):
    m = jnp.mean(x, axis=-1, keepdims=True)
    d = x - m
    v = jnp.mean(d * d, axis=-1, keepdims=True)
    return d / jnp.sqrt(v + _EPS)


def _gelu(x):
    c = 0.7978845608028654
    return 0.5 * x * (1.0 + jnp.tanh(c * (x + 0.044715 * (x * x * x))))


def _dot(a, b):
    return jnp.dot(a, b, preferred_element_type=_F32)


def _dot_t(a, b):
    return lax.dot_general(a, b, (((1,), (1,)), ((), ())), preferred_element_type=_F32)


def _pair_masks():
    row = lax.broadcasted_iota(jnp.int32, (8, _R), 0)
    col = lax.broadcasted_iota(jnp.int32, (8, _R), 1)
    own = (col >= row * _DH) & (col < (row + 1) * _DH)
    return own, col < _DH


_C2 = float(_DH) ** -0.5 * 1.4426950408889634


def _softmax_parts(s, first):
    m = jnp.max(s, axis=-1, keepdims=True)
    e = jnp.exp2(s - m)
    inv = 1.0 / jnp.sum(e, axis=-1, keepdims=True)
    return e, jnp.where(first, inv[0:1, :], inv[1:2, :])


def _layer2(xn8, always, kres, vres, wqres, wores, q_ref, s_ref, e_ref, inv_ref, lhs_ref, d_ref, acc_ref):
    own, first = _pair_masks()
    sub = lax.broadcasted_iota(jnp.int32, (8, 128), 0)
    lane = lax.broadcasted_iota(jnp.int32, (8, 128), 1)

    def tie(a, b):
        return jnp.where(always, a, b)

    def rows(i, n):
        return pl.ds(i * n, n) if isinstance(i, int) else pl.ds(pl.multiple_of(i * n, n), n)

    def q_unit(i, slot):
        q8 = _dot(xn8, pltpu.bitcast(wqres[:, rows(i, _R)], _BF))
        q_ref[slot] = jnp.where(own, q8 * _C2, 0.0)
        return q8[:, 0:128]

    def qk_unit(i, slot, c):
        cols = slice(c * _CK, (c + 1) * _CK)
        s = _dot(q_ref[slot].astype(_BF), pltpu.bitcast(kres[rows(i, _DH), cols], _BF))
        s_ref[slot, :, cols] = s
        return s[:, 0:128]

    def o_unit(i, lhs):
        r = _dot(lhs.astype(_BF), pltpu.bitcast(wores[rows(i, _DH), :], _BF))
        acc_ref[...] += r
        return r[:, 0:128]

    def softmax(slot):
        s = s_ref[slot]
        m = jnp.max(s, axis=-1, keepdims=True)
        e = jnp.exp2(s - m)
        inv = 1.0 / jnp.sum(e, axis=-1, keepdims=True)
        inv = jnp.where(first, inv[0:1, :], inv[1:2, :])
        e_ref[slot] = e
        inv_ref[slot] = inv
        return jnp.broadcast_to(m, (8, 128)), inv[:, 0:128]

    def fold_rows(a, red):
        a = jnp.broadcast_to(jnp.sum(a, axis=1, keepdims=True), a.shape)
        for b in range(a.shape[0] // 8):
            v, w = a[8 * b:8 * b + 8], 8
            while red and red[-1][0] == w and w < 128:
                v = jnp.where((lane & w) == 0, red.pop()[1], v)
                w *= 2
            red.append((w, v))
        return red[-1][1]

    def pv_unit(i, slot, hh, c, ties, red, defer=False):
        r0 = hh * _DH + c * _RV
        vrows = pl.ds(i * _R + r0, _RV) if isinstance(i, int) else pl.ds(pl.multiple_of(i * _R + r0, _RV), _RV)
        a = None
        for t in ties:
            a = tie(jnp.zeros((8, 128), _F32) if a is None else a, t)
        if a is not None:
            a = jnp.tile(a, (_RV // 8, 1))
        accs = [a] + [None] * (_NCH - 1)
        for j in range(_W // 128):
            p = jnp.broadcast_to(e_ref[slot, hh:hh + 1, j * 128:(j + 1) * 128], (8, 128))
            t = vres[vrows, j * 128:(j + 1) * 128].astype(_F32) * jnp.tile(p, (_RV // 8, 1))
            n = j // 2 % _NCH
            accs[n] = t if accs[n] is None else accs[n] + t
        a = accs[0]
        for t in accs[1:]:
            a = a + t
        if defer:
            d_ref[0:_RV, :] = a
            return a[0:8]
        return fold_rows(a, red)

    def px_unit(i, slot, c, ox, rx):
        cols = slice(c * _CKX, (c + 1) * _CKX)
        r0 = _R - rx
        vrows = pl.ds(i * _R + r0, rx) if isinstance(i, int) else pl.ds(pl.multiple_of(i * _R + r0, 32), rx)
        o = _dot_t(e_ref[slot, :, cols].astype(_BF), vres[vrows, cols])
        ox[0] = o if c == 0 else ox[0] + o
        return jnp.broadcast_to(o[:, 0:1], (8, 128))

    def make_lhs(slot, red, ox, rx):
        parts = [jnp.where((lane & 7) == sub, v, 0.0)[:, 0:w] for (w, v) in red]
        if rx:
            parts.append(jnp.where(own[:, _R - rx:], ox[0], 0.0))
        return jnp.concatenate(parts, axis=1) * inv_ref[slot]

    def park(red):
        for n, (_, v) in enumerate(red):
            d_ref[_RV + 8 * n:_RV + 8 * n + 8, :] = v

    def unpark(slot):
        widths = []
        for b in range((_R - _RV) // 8):
            w = 8
            while widths and widths[-1] == w and w < 128:
                widths.pop()
                w *= 2
            widths.append(w)
        red = [(w, d_ref[_RV + 8 * n:_RV + 8 * n + 8, :]) for n, w in enumerate(widths)]
        fold_rows(d_ref[0:_RV, :], red)
        return make_lhs(slot, red, None, 0)

    nck = _W // _CK
    nrv = _DH // _RV
    t_w, t_qk = 125, _R * _CK / 2048 * 1.03
    t_pv = _RV * _W / 2048 * _PVC
    _UN_T = t_pv * (_R - _RX) / _RV
    t_px = _CKX / 2048 * 2.05

    def step(i, par, mxu, carry=(), sm_after=0, rx=0, defer=False, parked=False, out=True, sm=True):
        def run_softmax(t0, t1):
            m, inv = softmax(1 - par)
            pending.extend([(t0, m), (t1, inv)])

        mxu = list(mxu)
        if out:
            lhs = unpark(1 - par) if parked else None
            mxu.insert(min(len(mxu), _OPOS), (t_w, lambda: o_unit(i - 1, lhs_ref[1 - par] if lhs is None else lhs)))
        ox = [None]
        mxu = [(t_px * rx, functools.partial(px_unit, i, par, c, ox, rx)) for c in range(_W // _CKX) if rx] + mxu
        mxu.reverse()
        pending = [(t - _UN_T, v) for (t, v) in carry]
        if sm and sm_after == 0:
            run_softmax(_SMA, _SMB)
        tm, n = 0.0, 0

        def run_mxu():
            nonlocal tm, n
            dt, f = mxu.pop()
            tm += dt
            n += 1
            pending.append((tm * _SLA + _SLK, f()))
            if sm and n == sm_after:
                run_softmax(tm + _SMP, tm + _SMQ)

        tv, red = float(_TV0), []
        for hh in range(2):
            for c in range(max(0, min(_DH, _R - rx - hh * _DH)) // _RV):
                while mxu and tm * _SLA + _SLK <= tv + 2 * t_pv + 200:
                    run_mxu()
                ties = [v for (t, v) in pending if t <= tv]
                pending[:] = [(t, v) for (t, v) in pending if t > tv]
                v = pv_unit(i, par, hh, c, ties, red, defer and hh == 1 and c == nrv - 1)
                tv += t_pv
                pending.append((tv + _RDL, v))
        while mxu:
            run_mxu()
        if defer:
            park(red)
        else:
            lhs_ref[par] = make_lhs(par, red, ox, rx)
        return pending

    def q_u(i, par):
        return [(t_w, functools.partial(q_unit, i, par))]

    def qk_u(i, par, lo=0, hi=nck):
        return [(t_qk, functools.partial(qk_unit, i, par, c)) for c in range(lo, hi)]

    acc_ref[...] = jnp.zeros_like(acc_ref)
    for _, f in q_u(0, 0) + q_u(1, 1) + qk_u(0, 0):
        f()
    softmax(0)
    ahead = (0,) + tuple(_AH) + (nck,)
    nr = len(ahead)
    assert (_NP - 3 - nr) % 2 == 0
    carry = ()
    for i in range(nr):
        par = i % 2
        lo, hi = ahead[i], ahead[min(i + 1, nr - 1)]
        mxu = qk_u(i + 1, 1 - par, lo) + q_u(i + 2, par) + qk_u(i + 2, par, 0, hi)
        if i == nr - 1:
            mxu = qk_u(i + 2, par) + q_u(i + 3, 1 - par)
        elif i == nr - 2:
            mxu = mxu + q_u(i + 3, 1 - par)
        carry = step(i, par, mxu, carry, 0 if i == nr - 1 else nck - lo, out=i > 0, defer=True, parked=i > 0)

    @pl.loop(0, (_NP - 3 - nr) // 2)
    def _(n):
        carry = ()
        for u in (nr, nr + 1):
            i, par = 2 * n + u, u % 2
            carry = step(i, par, qk_u(i + 2, par) + q_u(i + 3, 1 - par), carry, defer=True, parked=True)

    n = _NP - 3
    carry = step(n, n % 2, qk_u(n + 2, n % 2), (), parked=True)
    carry = step(n + 1, (n + 1) % 2, [], carry, rx=_RXA)
    carry = step(n + 2, (n + 2) % 2, [], carry, rx=_RXB, sm=False)
    o_unit(n + 2, lhs_ref[(n + 2) % 2])


def _kernel(x_hbm, k_hbm, v_hbm, wq_hbm, wo_hbm, w3_hbm, w4_hbm, o_ref,
            kland, kres, vres, wqland, wqres, woland, wores, w3buf, w4buf, acc_ref,
            q_ref, s_ref, e_ref, inv_ref, lhs_ref, d_ref, x_ref, sem_k, sem_v, sem_q, sem_o, sem_w, *, sk):
    def k_copy(i):
        return pltpu.make_async_copy(
            k_hbm.at[pl.ds(i * _R, _R), pl.ds(sk - _W, _W)],
            kland.at[i % _NLAND], sem_k.at[i % _NLAND])

    def v_copy(i):
        return pltpu.make_async_copy(
            v_hbm.at[pl.ds(i * _R, _R), pl.ds(sk - _W, _W)],
            vres.at[pl.ds(i * _R, _R), :], sem_v.at[i % (_VAHEAD + 1)])

    if _WU32:
        def wq_copy(i):
            return pltpu.make_async_copy(
                wq_hbm.at[:, pl.ds(i * _R, _R)], wqland.at[i % 2], sem_q.at[i % 2])

        def wo_copy(i):
            return pltpu.make_async_copy(
                wo_hbm.at[pl.ds(i * _R, _R), :], woland.at[i % 2], sem_o.at[i % 2])

        def wq_of(i):
            return pltpu.bitcast(wqres[:, i * _R:(i + 1) * _R], _BF)

        def wo_of(i):
            return pltpu.bitcast(wores[i * _DH:(i + 1) * _DH, :], _BF)
    else:
        def wq_copy(i):
            return pltpu.make_async_copy(
                wq_hbm.at[:, pl.ds(i * _R, _R)], wqres.at[:, pl.ds(i * _R, _R)], sem_q.at[i])

        def wo_copy(i):
            return pltpu.make_async_copy(
                wo_hbm.at[pl.ds(i * _R, _R), :], wores.at[pl.ds(i * _R, _R), :], sem_o.at[i])

        def wq_of(i):
            return wqres[:, i * _R:(i + 1) * _R]

        def wo_of(i):
            return wores[i * _R:(i + 1) * _R, :]

    w3_copy = pltpu.make_async_copy(w3_hbm, w3buf.at[:, pl.ds(0, _F)], sem_w.at[0])
    fc = _F // _NW4
    w4_copies = [pltpu.make_async_copy(w4_hbm.at[pl.ds(n * fc, fc), :], w4buf.at[pl.ds(n * fc, fc), :], sem_w.at[1 + n]) for n in range(_NW4)]
    x_copy = pltpu.make_async_copy(x_hbm, x_ref, sem_w.at[0])

    def start_pair(i):
        wq_copy(i).start()
        k_copy(i).start()
        wo_copy(i).start()

    for i in range(_NLAND):
        start_pair(i)
        if i < _VAHEAD:
            v_copy(i).start()
        if i == 0:
            x_copy.start()

    own, first = _pair_masks()

    def mlp_in(x):
        y = _layernorm(x)
        my = jnp.mean(y, axis=-1, keepdims=True)
        vy = jnp.mean(y * y, axis=-1, keepdims=True) - my * my
        yn = (y - my) / jnp.sqrt(vy + _EPS)
        yn = jnp.broadcast_to(yn, (8, _D)).astype(_BF)
        h = _gelu(_dot(yn, w3buf[:, 0:_F])).astype(_BF)
        return y, h

    def mlp_out(x, y, h, wait=False):
        out = x + y
        for n in range(_NW4):
            if wait:
                w4_copies[n].wait()
            out = out + _dot(h[:, n * fc:(n + 1) * fc], w4buf[n * fc:(n + 1) * fc, :])[0:1]
        return out

    x_copy.wait()
    x = x_ref[...].astype(_F32)
    always = ~(jnp.abs(jnp.broadcast_to(x[:, 0:128], (8, 128))) < 0.0)
    xn8 = jnp.broadcast_to(_layernorm(x), (8, _D)).astype(_BF)
    acc_ref[...] = jnp.zeros_like(acc_ref)

    @pl.loop(0, _NP)
    def _(i):
        wq_copy(i).wait()
        k_copy(i).wait()
        wo_copy(i).wait()
        v_copy(i).wait()

        @pl.when(i + _VAHEAD < _NP)
        def _():
            v_copy(i + _VAHEAD).start()

        rk = pl.multiple_of(i * _DH, _DH)
        rv = pl.multiple_of(i * _R, _R)
        if _WU32:
            wq = wqland[i % 2]
            wo = woland[i % 2]
            wqres[:, pl.ds(rv, _R)] = pltpu.bitcast(wq, _U32)
            wores[pl.ds(rk, _DH), :] = pltpu.bitcast(wo, _U32)
        else:
            wq = wqres[:, pl.ds(rv, _R)]
            wo = wores[pl.ds(rv, _R), :]
        q = jnp.where(own, _dot(xn8, wq) * _C2, 0.0).astype(_BF)
        k = kland[i % _NLAND]
        kres[pl.ds(rk, _DH), :] = pltpu.bitcast(k, _U32)
        e, inv = _softmax_parts(_dot(q, k), first)
        o = _dot_t(e.astype(_BF), vres[pl.ds(rv, _R), :])
        lhs = (jnp.where(own, o, 0.0) * inv).astype(_BF)
        acc_ref[...] += _dot(lhs, wo)

        @pl.when(i + _NLAND < _NP)
        def _():
            start_pair(i + _NLAND)

        @pl.when(i + _NLAND == _NP)
        def _():
            w3_copy.start()
            for c in w4_copies:
                c.start()

    x = x + jnp.sum(acc_ref[...], axis=0, keepdims=True)
    w3_copy.wait()
    y, h = mlp_in(x)
    x = mlp_out(x, y, h, wait=True)

    xn8 = jnp.broadcast_to(_layernorm(x), (8, _D)).astype(_BF)
    _layer2(xn8, always, kres, vres, wqres, wores, q_ref, s_ref, e_ref, inv_ref, lhs_ref, d_ref, acc_ref)
    x = x + jnp.sum(acc_ref[...], axis=0, keepdims=True)
    y, h = mlp_in(x)
    x = mlp_out(x, y, h)
    o_ref[...] = x.astype(o_ref.dtype)


@jax.jit
def pallas_interleave_layers__sliding_block_cached__mixer_s_mlp__decode_kernel(
    A_x: jax.Array,
    A_k_cache: jax.Array,
    A_v_cache: jax.Array,
    A_wq: jax.Array,
    A_wo: jax.Array,
    B_x: jax.Array,
    B_w1: jax.Array,
    B_w2: jax.Array,
    B_w3: jax.Array,
    B_w4: jax.Array,
):
    del B_x, B_w1, B_w2
    _, hkv, sk, dh = A_k_cache.shape
    assert (hkv, dh) == (_H, _DH) and min(4096, max(256, sk // 4)) == _W
    kt = jnp.swapaxes(A_k_cache, 2, 3).reshape(_H * _DH, sk)
    vt = jnp.swapaxes(A_v_cache, 2, 3).reshape(_H * _DH, sk)
    any_spec = pl.BlockSpec(memory_space=pl.ANY)
    if _WU32:
        w_scratch = [
            pltpu.VMEM((2, _D, _R), _BF), pltpu.VMEM((_D // 2, _H * _DH), _U32),
            pltpu.VMEM((2, _R, _D), _BF), pltpu.VMEM((_H * _DH // 2, _D), _U32),
        ]
    else:
        w_scratch = [
            pltpu.VMEM((8, 128), _BF), pltpu.VMEM((_D, _H * _DH + _PAD), _BF),
            pltpu.VMEM((8, 128), _BF), pltpu.VMEM((_H * _DH, _D), _BF),
        ]
    out = pl.pallas_call(
        functools.partial(_kernel, sk=sk),
        out_shape=jax.ShapeDtypeStruct((1, _D), A_x.dtype),
        in_specs=[any_spec] * 7,
        out_specs=pl.BlockSpec(memory_space=pltpu.VMEM),
        scratch_shapes=[
            pltpu.VMEM((_NLAND, _R, _W), _BF),
            pltpu.VMEM((_H * _DH // 2, _W), _U32),
            pltpu.VMEM((_H * _DH, _W), _BF),
            *w_scratch,
            pltpu.VMEM((_D, _F + _PAD), _BF),
            pltpu.VMEM((_F, _D), _BF),
            pltpu.VMEM((8, _D), _F32),
            pltpu.VMEM((2, 8, _R), _F32),
            pltpu.VMEM((2, 8, _W), _F32),
            pltpu.VMEM((2, 8, _W), _F32),
            pltpu.VMEM((2, 8, _R), _F32),
            pltpu.VMEM((2, 8, _R), _F32),
            pltpu.VMEM((_RV + 64, 128), _F32),
            pltpu.VMEM((1, _D), _BF),
            pltpu.SemaphoreType.DMA((_NLAND,)),
            pltpu.SemaphoreType.DMA((_VAHEAD + 1,)),
            pltpu.SemaphoreType.DMA((2,)),
            pltpu.SemaphoreType.DMA((2,)),
            pltpu.SemaphoreType.DMA((1 + _NW4,)),
        ],
        compiler_params=pltpu.CompilerParams(vmem_limit_bytes=127 * 1024 * 1024, flags=_FLAGS[_FL]),
        name="interleave_decode",
    )(A_x.reshape(1, _D), kt, vt, A_wq, A_wo, B_w3, B_w4)
    return out.reshape(1, 1, _D)
```

```python
import functools

import jax
import jax.numpy as jnp
import jax.experimental.pallas as pl
import jax.experimental.pallas.tpu as pltpu
from jax import lax

_H = 32
_DH = 192
_W = 4096
_D = 640
_F = 1536
_EPS = 1e-5
_BF = jnp.bfloat16
_F32 = jnp.float32
_U32 = jnp.uint32

_NP = _H // 2
_R = 2 * _DH
_NW4 = 3
_C2 = float(_DH) ** -0.5 * 1.4426950408889634

_CK = 512
_CX = 1024
_RV = 32
_RX = 192
_RAMP = 6
_T_W = 125.0
_T_QK = _R * _CK / 2048 * 1.03
_T_PX = _RX * _CX / 2048 * 2.05
_T_PV = _RV * _W / 2048 * 1.6
_T_STEP = _T_PV * _R / _RV
_T_MXU = 40.0
_T_START = 40.0
_T_MAX = 150.0
_T_SUM = 900.0
_T_SUM_RAMP = 450.0
_T_FOLD = 900.0


def _layernorm(x):
    m = jnp.mean(x, axis=-1, keepdims=True)
    d = x - m
    v = jnp.mean(d * d, axis=-1, keepdims=True)
    return d / jnp.sqrt(v + _EPS)


def _layernorm_centred(y):
    m = jnp.mean(y, axis=-1, keepdims=True)
    v = jnp.mean(y * y, axis=-1, keepdims=True) - m * m
    return (y - m) / jnp.sqrt(v + _EPS)


def _gelu(x):
    c = 0.7978845608028654
    return 0.5 * x * (1.0 + jnp.tanh(c * (x + 0.044715 * (x * x * x))))


def _dot(a, b):
    return jnp.dot(a, b, preferred_element_type=_F32)


def _dot_t(a, b):
    return lax.dot_general(a, b, (((1,), (1,)), ((), ())), preferred_element_type=_F32)


def _pair_masks():
    row = lax.broadcasted_iota(jnp.int32, (8, _R), 0)
    col = lax.broadcasted_iota(jnp.int32, (8, _R), 1)
    own = (col >= row * _DH) & (col < (row + 1) * _DH)
    return own, col < _DH


def _softmax_parts(s, first):
    m = jnp.max(s, axis=-1, keepdims=True)
    e = jnp.exp2(s - m)
    inv = 1.0 / jnp.sum(e, axis=-1, keepdims=True)
    return e, m, jnp.where(first, inv[0:1, :], inv[1:2, :])


def _layer2(xn8, always, kres, vres, wqres, wores,
            q_ref, s_ref, e_ref, inv_ref, lhs_ref, d_ref, acc_ref):
    own, first = _pair_masks()
    sub = lax.broadcasted_iota(jnp.int32, (8, 128), 0)
    lane = lax.broadcasted_iota(jnp.int32, (8, 128), 1)
    nck = _W // _CK
    nrv = _DH // _RV

    def tie(a, b):
        return jnp.where(always, a, b)

    def span(start, n, align):
        return pl.ds(start if isinstance(start, int) else pl.multiple_of(start, align), n)

    def q_unit(i, slot):
        q8 = _dot(xn8, pltpu.bitcast(wqres[:, span(i * _R, _R, _R)], _BF))
        q_ref[slot] = jnp.where(own, q8 * _C2, 0.0)
        return q8[:, 0:128]

    def qk_unit(i, slot, c):
        cols = slice(c * _CK, (c + 1) * _CK)
        k = pltpu.bitcast(kres[span(i * _DH, _DH, _DH), cols], _BF)
        s = _dot(q_ref[slot].astype(_BF), k)
        s_ref[slot, :, cols] = s
        return s[:, 0:128]

    def o_unit(i, lhs):
        r = _dot(lhs.astype(_BF), pltpu.bitcast(wores[span(i * _DH, _DH, _DH), :], _BF))
        acc_ref[...] += r
        return r[:, 0:128]

    def px_unit(i, slot, c, ox):
        cols = slice(c * _CX, (c + 1) * _CX)
        o = _dot_t(e_ref[slot, :, cols].astype(_BF), vres[pl.ds((i + 1) * _R - _RX, _RX), cols])
        ox[0] = o if c == 0 else ox[0] + o
        return jnp.broadcast_to(o[:, 0:1], (8, 128))

    def softmax(slot):
        e, m, inv = _softmax_parts(s_ref[slot], first)
        e_ref[slot] = e
        inv_ref[slot] = inv
        return jnp.broadcast_to(m, (8, 128)), inv[:, 0:128]

    def fold(a, red):
        a = jnp.broadcast_to(jnp.sum(a, axis=1, keepdims=True), a.shape)
        for b in range(a.shape[0] // 8):
            v, w = a[8 * b:8 * b + 8], 8
            while red and red[-1][0] == w and w < 128:
                v = jnp.where((lane & w) == 0, red.pop()[1], v)
                w *= 2
            red.append((w, v))
        return red[-1][1]

    def pv_unit(i, slot, hh, c, ties, red, park):
        rows = span(i * _R + hh * _DH + c * _RV, _RV, _RV)
        a = None
        for t in ties:
            a = tie(jnp.zeros((8, 128), _F32) if a is None else a, t)
        if a is not None:
            a = jnp.tile(a, (_RV // 8, 1))
        accs = [a, None]
        for j in range(_W // 128):
            cols = slice(j * 128, (j + 1) * 128)
            p = jnp.broadcast_to(e_ref[slot, hh:hh + 1, cols], (8, 128))
            t = vres[rows, cols].astype(_F32) * jnp.tile(p, (_RV // 8, 1))
            n = j // 2 % 2
            accs[n] = t if accs[n] is None else accs[n] + t
        a = accs[0] + accs[1]
        if park:
            d_ref[0:_RV, :] = a
            return a[0:8]
        return fold(a, red)

    def make_lhs(slot, red, ox=None):
        parts = [jnp.where((lane & 7) == sub, v, 0.0)[:, 0:w] for (w, v) in red]
        if ox is not None:
            parts.append(jnp.where(own[:, _R - _RX:], ox[0], 0.0))
        return jnp.concatenate(parts, axis=1) * inv_ref[slot]

    def unpark(slot):
        widths = []
        for _ in range((_R - _RV) // 8):
            w = 8
            while widths and widths[-1] == w and w < 128:
                widths.pop()
                w *= 2
            widths.append(w)
        red = [(w, d_ref[_RV + 8 * n:_RV + 8 * n + 8, :]) for n, w in enumerate(widths)]
        fold(d_ref[0:_RV, :], red)
        return make_lhs(slot, red)

    def step(i, par, mxu, carry, *, sm_after=0, sm=True, out=True, parked=True, park=True, px=False):
        mxu = list(mxu)
        if out:
            lhs = unpark(1 - par) if parked else None
            mxu.append((_T_W, lambda: o_unit(i - 1, lhs_ref[1 - par] if lhs is None else lhs)))
        ox = [None]
        if px:
            mxu = [(_T_PX, functools.partial(px_unit, i, par, c, ox)) for c in range(_W // _CX)] + mxu
        mxu.reverse()
        pending = [(t - _T_STEP, v) for (t, v) in carry]
        if sm and sm_after == 0:
            pending += zip((_T_MAX, _T_SUM), softmax(1 - par))
        tm, done = 0.0, 0

        def run_mxu():
            nonlocal tm, done
            dt, fn = mxu.pop()
            tm += dt
            done += 1
            pending.append((tm + _T_MXU, fn()))
            if sm and done == sm_after:
                pending.extend(zip((tm + _T_MAX, tm + _T_SUM_RAMP), softmax(1 - par)))

        tv, red = _T_START, []
        for hh in range(2):
            for c in range(0 if px and hh else nrv):
                while mxu and tm + _T_MXU <= tv + 2 * _T_PV + 200:
                    run_mxu()
                ties = [v for (t, v) in pending if t <= tv]
                pending[:] = [(t, v) for (t, v) in pending if t > tv]
                v = pv_unit(i, par, hh, c, ties, red, park and hh == 1 and c == nrv - 1)
                tv += _T_PV
                pending.append((tv + _T_FOLD, v))
        while mxu:
            run_mxu()
        if park:
            for n, (_, v) in enumerate(red):
                d_ref[_RV + 8 * n:_RV + 8 * n + 8, :] = v
        else:
            lhs_ref[par] = make_lhs(par, red, ox if px else None)
        return pending

    def q(i, par):
        return [(_T_W, functools.partial(q_unit, i, par))]

    def qk(i, par, lo=0, hi=nck):
        return [(_T_QK, functools.partial(qk_unit, i, par, c)) for c in range(lo, hi)]

    acc_ref[...] = jnp.zeros_like(acc_ref)
    for _, fn in q(0, 0) + q(1, 1) + qk(0, 0):
        fn()
    softmax(0)
    carry = step(0, 0, qk(1, 1) + q(2, 0) + qk(2, 0, 0, _RAMP), (),
                 sm_after=nck, out=False)
    carry = step(1, 1, qk(2, 0, _RAMP) + q(3, 1) + qk(3, 1) + q(4, 0), carry,
                 sm_after=nck - _RAMP)
    carry = step(2, 0, qk(4, 0) + q(5, 1), carry)

    @pl.loop(0, (_NP - 6) // 2)
    def _(n):
        carry = ()
        for u in (3, 4):
            i, par = 2 * n + u, u % 2
            carry = step(i, par, qk(i + 2, par) + q(i + 3, 1 - par), carry)

    n = _NP - 3
    carry = step(n, 1, qk(n + 2, 1), (), park=False)
    carry = step(n + 1, 0, [], carry, parked=False, park=False, px=True)
    carry = step(n + 2, 1, [], carry, parked=False, park=False, px=True, sm=False)
    o_unit(n + 2, lhs_ref[1])


def _kernel(x_hbm, k_hbm, v_hbm, wq_hbm, wo_hbm, w3_hbm, w4_hbm, o_ref,
            kland, kres, vres, wqland, wqres, woland, wores, w3buf, w4buf, acc_ref,
            q_ref, s_ref, e_ref, inv_ref, lhs_ref, d_ref, x_ref,
            sem_k, sem_v, sem_q, sem_o, sem_w, *, sk):
    def k_copy(i):
        return pltpu.make_async_copy(
            k_hbm.at[pl.ds(i * _R, _R), pl.ds(sk - _W, _W)], kland.at[i % 2], sem_k.at[i % 2])

    def wq_copy(i):
        return pltpu.make_async_copy(
            wq_hbm.at[:, pl.ds(i * _R, _R)], wqland.at[i % 2], sem_q.at[i % 2])

    def wo_copy(i):
        return pltpu.make_async_copy(
            wo_hbm.at[pl.ds(i * _R, _R), :], woland.at[i % 2], sem_o.at[i % 2])

    def v_copy(i):
        return pltpu.make_async_copy(
            v_hbm.at[pl.ds(i * _R, _R), pl.ds(sk - _W, _W)],
            vres.at[pl.ds(i * _R, _R), :], sem_v.at[i % 3])

    def start_pair(i):
        wq_copy(i).start()
        k_copy(i).start()
        wo_copy(i).start()

    fc = _F // _NW4
    x_copy = pltpu.make_async_copy(x_hbm, x_ref, sem_w.at[0])
    w3_copy = pltpu.make_async_copy(w3_hbm, w3buf.at[:, pl.ds(0, _F)], sem_w.at[0])
    w4_copies = [
        pltpu.make_async_copy(w4_hbm.at[pl.ds(n * fc, fc), :], w4buf.at[pl.ds(n * fc, fc), :],
                              sem_w.at[1 + n])
        for n in range(_NW4)
    ]

    def mlp_hidden(x):
        y = _layernorm(x)
        yn = jnp.broadcast_to(_layernorm_centred(y), (8, _D)).astype(_BF)
        return y, _gelu(_dot(yn, w3buf[:, 0:_F])).astype(_BF)

    def mlp_out(x, y, h, wait):
        out = x + y
        for n in range(_NW4):
            if wait:
                w4_copies[n].wait()
            out = out + _dot(h[:, n * fc:(n + 1) * fc], w4buf[n * fc:(n + 1) * fc, :])[0:1]
        return out

    start_pair(0)
    v_copy(0).start()
    x_copy.start()
    start_pair(1)
    v_copy(1).start()

    own, first = _pair_masks()
    x_copy.wait()
    x = x_ref[...].astype(_F32)
    always = ~(jnp.abs(jnp.broadcast_to(x[:, 0:128], (8, 128))) < 0.0)
    xn8 = jnp.broadcast_to(_layernorm(x), (8, _D)).astype(_BF)
    acc_ref[...] = jnp.zeros_like(acc_ref)

    @pl.loop(0, _NP)
    def _(i):
        wq_copy(i).wait()
        k_copy(i).wait()
        wo_copy(i).wait()
        v_copy(i).wait()

        @pl.when(i + 2 < _NP)
        def _():
            v_copy(i + 2).start()

        half = pl.multiple_of(i * _DH, _DH)
        full = pl.multiple_of(i * _R, _R)
        wq = wqland[i % 2]
        wo = woland[i % 2]
        wqres[:, pl.ds(full, _R)] = pltpu.bitcast(wq, _U32)
        wores[pl.ds(half, _DH), :] = pltpu.bitcast(wo, _U32)
        q = jnp.where(own, _dot(xn8, wq) * _C2, 0.0).astype(_BF)
        k = kland[i % 2]
        kres[pl.ds(half, _DH), :] = pltpu.bitcast(k, _U32)
        e, _, inv = _softmax_parts(_dot(q, k), first)
        o = _dot_t(e.astype(_BF), vres[pl.ds(full, _R), :])
        acc_ref[...] += _dot((jnp.where(own, o, 0.0) * inv).astype(_BF), wo)

        @pl.when(i + 2 < _NP)
        def _():
            start_pair(i + 2)

        @pl.when(i + 2 == _NP)
        def _():
            w3_copy.start()
            for c in w4_copies:
                c.start()

    x = x + jnp.sum(acc_ref[...], axis=0, keepdims=True)
    w3_copy.wait()
    y, h = mlp_hidden(x)
    x = mlp_out(x, y, h, wait=True)

    xn8 = jnp.broadcast_to(_layernorm(x), (8, _D)).astype(_BF)
    _layer2(xn8, always, kres, vres, wqres, wores,
            q_ref, s_ref, e_ref, inv_ref, lhs_ref, d_ref, acc_ref)
    x = x + jnp.sum(acc_ref[...], axis=0, keepdims=True)
    y, h = mlp_hidden(x)
    o_ref[...] = mlp_out(x, y, h, wait=False).astype(o_ref.dtype)


@jax.jit
def pallas_interleave_layers__sliding_block_cached__mixer_s_mlp__decode_kernel(
    A_x: jax.Array,
    A_k_cache: jax.Array,
    A_v_cache: jax.Array,
    A_wq: jax.Array,
    A_wo: jax.Array,
    B_x: jax.Array,
    B_w1: jax.Array,
    B_w2: jax.Array,
    B_w3: jax.Array,
    B_w4: jax.Array,
):
    del B_x, B_w1, B_w2
    _, hkv, sk, dh = A_k_cache.shape
    assert A_x.shape == (1, 1, _D) and (hkv, dh) == (_H, _DH)
    assert min(4096, max(256, sk // 4)) == _W
    kt = jnp.swapaxes(A_k_cache, 2, 3).reshape(_H * _DH, sk)
    vt = jnp.swapaxes(A_v_cache, 2, 3).reshape(_H * _DH, sk)
    out = pl.pallas_call(
        functools.partial(_kernel, sk=sk),
        out_shape=jax.ShapeDtypeStruct((1, _D), A_x.dtype),
        in_specs=[pl.BlockSpec(memory_space=pl.ANY)] * 7,
        out_specs=pl.BlockSpec(memory_space=pltpu.VMEM),
        scratch_shapes=[
            pltpu.VMEM((2, _R, _W), _BF),
            pltpu.VMEM((_H * _DH // 2, _W), _U32),
            pltpu.VMEM((_H * _DH, _W), _BF),
            pltpu.VMEM((2, _D, _R), _BF),
            pltpu.VMEM((_D // 2, _H * _DH), _U32),
            pltpu.VMEM((2, _R, _D), _BF),
            pltpu.VMEM((_H * _DH // 2, _D), _U32),
            pltpu.VMEM((_D, _F + 128), _BF),
            pltpu.VMEM((_F, _D), _BF),
            pltpu.VMEM((8, _D), _F32),
            pltpu.VMEM((2, 8, _R), _F32),
            pltpu.VMEM((2, 8, _W), _F32),
            pltpu.VMEM((2, 8, _W), _F32),
            pltpu.VMEM((2, 8, _R), _F32),
            pltpu.VMEM((2, 8, _R), _F32),
            pltpu.VMEM((_RV + 64, 128), _F32),
            pltpu.VMEM((1, _D), _BF),
            pltpu.SemaphoreType.DMA((2,)),
            pltpu.SemaphoreType.DMA((3,)),
            pltpu.SemaphoreType.DMA((2,)),
            pltpu.SemaphoreType.DMA((2,)),
            pltpu.SemaphoreType.DMA((1 + _NW4,)),
        ],
        compiler_params=pltpu.CompilerParams(vmem_limit_bytes=127 * 1024 * 1024),
        name="interleave_decode",
    )(A_x.reshape(1, _D), kt, vt, A_wq, A_wo, B_w3, B_w4)
    return out.reshape(1, 1, _D)
```

```python
import functools

import jax
import jax.numpy as jnp
import jax.experimental.pallas as pl
import jax.experimental.pallas.tpu as pltpu
from jax import lax

_H = 32
_DH = 192
_W = 4096
_D = 640
_F = 1536
_EPS = 1e-5
_BF = jnp.bfloat16
_F32 = jnp.float32
_U32 = jnp.uint32

_NP = _H // 2
_R = 2 * _DH
_W4 = (0, 768, 1280, 1536)
_NW4 = len(_W4) - 1
_C2 = float(_DH) ** -0.5 * 1.4426950408889634

_CK = 512
_CX = 1024
_RV = 32
_RX = 192
_RAMP = 6
_T_W = 125.0
_T_QK = _R * _CK / 2048 * 1.03
_T_PX = _RX * _CX / 2048 * 2.05
_T_PV = _RV * _W / 2048 * 1.6
_T_STEP = _T_PV * _R / _RV
_T_MXU = 40.0
_T_START = 40.0
_T_MAX = 150.0
_T_SUM = 900.0
_T_SUM_RAMP = 450.0
_T_FOLD = 900.0


def _layernorm(x):
    m = jnp.mean(x, axis=-1, keepdims=True)
    d = x - m
    v = jnp.mean(d * d, axis=-1, keepdims=True)
    return d / jnp.sqrt(v + _EPS)


def _layernorm_near(x, c):
    d = x - c
    m = jnp.mean(d, axis=-1, keepdims=True)
    v = jnp.mean(d * d, axis=-1, keepdims=True) - m * m
    return (d - m) / jnp.sqrt(jnp.maximum(v, 0.0) + _EPS), c + m


def _gelu(x):
    c = 0.7978845608028654
    return 0.5 * x * (1.0 + jnp.tanh(c * (x + 0.044715 * (x * x * x))))


def _dot(a, b):
    return jnp.dot(a, b, preferred_element_type=_F32)


def _dot_t(a, b):
    return lax.dot_general(a, b, (((1,), (1,)), ((), ())), preferred_element_type=_F32)


def _pair_masks():
    row = lax.broadcasted_iota(jnp.int32, (8, _R), 0)
    col = lax.broadcasted_iota(jnp.int32, (8, _R), 1)
    own = (col >= row * _DH) & (col < (row + 1) * _DH)
    return own, col < _DH


def _softmax_parts(s, first):
    m = jnp.max(s, axis=-1, keepdims=True)
    e = jnp.exp2(s - m)
    inv = 1.0 / jnp.sum(e, axis=-1, keepdims=True)
    return e, m, jnp.where(first, inv[0:1, :], inv[1:2, :])


def _layer2(xn8, always, kres, vres, wqres, wores,
            q_ref, s_ref, e_ref, inv_ref, lhs_ref, d_ref, acc_ref):
    own, first = _pair_masks()
    sub = lax.broadcasted_iota(jnp.int32, (8, 128), 0)
    lane = lax.broadcasted_iota(jnp.int32, (8, 128), 1)
    nck = _W // _CK
    nrv = _DH // _RV

    def tie(a, b):
        return jnp.where(always, a, b)

    def span(start, n, align):
        return pl.ds(start if isinstance(start, int) else pl.multiple_of(start, align), n)

    def q_unit(i, slot):
        q8 = _dot(xn8, pltpu.bitcast(wqres[:, span(i * _R, _R, _R)], _BF))
        q_ref[slot] = jnp.where(own, q8 * _C2, 0.0)
        return q8[:, 0:128]

    def qk_unit(i, slot, c):
        cols = slice(c * _CK, (c + 1) * _CK)
        k = pltpu.bitcast(kres[span(i * _DH, _DH, _DH), cols], _BF)
        s = _dot(q_ref[slot].astype(_BF), k)
        s_ref[slot, :, cols] = s
        return s[:, 0:128]

    def o_unit(i, lhs):
        r = _dot(lhs.astype(_BF), pltpu.bitcast(wores[span(i * _DH, _DH, _DH), :], _BF))
        acc_ref[...] += r
        return r[:, 0:128]

    def px_unit(i, slot, c, ox):
        cols = slice(c * _CX, (c + 1) * _CX)
        o = _dot_t(e_ref[slot, :, cols].astype(_BF), vres[pl.ds((i + 1) * _R - _RX, _RX), cols])
        ox[0] = o if c == 0 else ox[0] + o
        return jnp.broadcast_to(o[:, 0:1], (8, 128))

    def softmax(slot):
        e, m, inv = _softmax_parts(s_ref[slot], first)
        e_ref[slot] = e
        inv_ref[slot] = inv
        return jnp.broadcast_to(m, (8, 128)), inv[:, 0:128]

    def fold(a, red):
        a = jnp.broadcast_to(jnp.sum(a, axis=1, keepdims=True), a.shape)
        for b in range(a.shape[0] // 8):
            v, w = a[8 * b:8 * b + 8], 8
            while red and red[-1][0] == w and w < 128:
                v = jnp.where((lane & w) == 0, red.pop()[1], v)
                w *= 2
            red.append((w, v))
        return red[-1][1]

    def pv_unit(i, slot, hh, c, ties, red, park):
        rows = span(i * _R + hh * _DH + c * _RV, _RV, _RV)
        a = None
        for t in ties:
            a = tie(jnp.zeros((8, 128), _F32) if a is None else a, t)
        if a is not None:
            a = jnp.tile(a, (_RV // 8, 1))
        accs = [a, None]
        for j in range(_W // 128):
            cols = slice(j * 128, (j + 1) * 128)
            p = jnp.broadcast_to(e_ref[slot, hh:hh + 1, cols], (8, 128))
            t = vres[rows, cols].astype(_F32) * jnp.tile(p, (_RV // 8, 1))
            n = j // 2 % 2
            accs[n] = t if accs[n] is None else accs[n] + t
        a = accs[0] + accs[1]
        if park:
            d_ref[0:_RV, :] = a
            return a[0:8]
        return fold(a, red)

    def make_lhs(slot, red, ox=None):
        parts = [jnp.where((lane & 7) == sub, v, 0.0)[:, 0:w] for (w, v) in red]
        if ox is not None:
            parts.append(jnp.where(own[:, _R - _RX:], ox[0], 0.0))
        return jnp.concatenate(parts, axis=1) * inv_ref[slot]

    def unpark(slot):
        widths = []
        for _ in range((_R - _RV) // 8):
            w = 8
            while widths and widths[-1] == w and w < 128:
                widths.pop()
                w *= 2
            widths.append(w)
        red = [(w, d_ref[_RV + 8 * n:_RV + 8 * n + 8, :]) for n, w in enumerate(widths)]
        fold(d_ref[0:_RV, :], red)
        return make_lhs(slot, red)

    def step(i, par, mxu, carry, *, sm_after=0, sm=True, out=True, parked=True, park=True, px=False):
        mxu = list(mxu)
        if out:
            lhs = unpark(1 - par) if parked else None
            mxu.append((_T_W, lambda: o_unit(i - 1, lhs_ref[1 - par] if lhs is None else lhs)))
        ox = [None]
        if px:
            mxu = [(_T_PX, functools.partial(px_unit, i, par, c, ox)) for c in range(_W // _CX)] + mxu
        mxu.reverse()
        pending = [(t - _T_STEP, v) for (t, v) in carry]
        if sm and sm_after == 0:
            pending += zip((_T_MAX, _T_SUM), softmax(1 - par))
        tm, done = 0.0, 0

        def run_mxu():
            nonlocal tm, done
            dt, fn = mxu.pop()
            tm += dt
            done += 1
            pending.append((tm + _T_MXU, fn()))
            if sm and done == sm_after:
                pending.extend(zip((tm + _T_MAX, tm + _T_SUM_RAMP), softmax(1 - par)))

        tv, red = _T_START, []
        for hh in range(2):
            for c in range(0 if px and hh else nrv):
                while mxu and tm + _T_MXU <= tv + 2 * _T_PV + 200:
                    run_mxu()
                ties = [v for (t, v) in pending if t <= tv]
                pending[:] = [(t, v) for (t, v) in pending if t > tv]
                v = pv_unit(i, par, hh, c, ties, red, park and hh == 1 and c == nrv - 1)
                tv += _T_PV
                pending.append((tv + _T_FOLD, v))
        while mxu:
            run_mxu()
        if park:
            for n, (_, v) in enumerate(red):
                d_ref[_RV + 8 * n:_RV + 8 * n + 8, :] = v
        else:
            lhs_ref[par] = make_lhs(par, red, ox if px else None)
        return pending

    def q(i, par):
        return [(_T_W, functools.partial(q_unit, i, par))]

    def qk(i, par, lo=0, hi=nck):
        return [(_T_QK, functools.partial(qk_unit, i, par, c)) for c in range(lo, hi)]

    acc_ref[...] = jnp.zeros_like(acc_ref)
    for _, fn in q(0, 0) + q(1, 1) + qk(0, 0):
        fn()
    softmax(0)
    carry = step(0, 0, qk(1, 1) + q(2, 0) + qk(2, 0, 0, _RAMP), (),
                 sm_after=nck, out=False)
    carry = step(1, 1, qk(2, 0, _RAMP) + q(3, 1) + qk(3, 1) + q(4, 0), carry,
                 sm_after=nck - _RAMP)
    carry = step(2, 0, qk(4, 0) + q(5, 1), carry)

    @pl.loop(0, (_NP - 6) // 2)
    def _(n):
        carry = ()
        for u in (3, 4):
            i, par = 2 * n + u, u % 2
            carry = step(i, par, qk(i + 2, par) + q(i + 3, 1 - par), carry)

    n = _NP - 3
    carry = step(n, 1, qk(n + 2, 1), (), park=False)
    carry = step(n + 1, 0, [], carry, parked=False, park=False, px=True)
    carry = step(n + 2, 1, [], carry, parked=False, park=False, px=True, sm=False)
    o_unit(n + 2, lhs_ref[1])


def _kernel(x_hbm, k_hbm, v_hbm, wq_hbm, wo_hbm, w3_hbm, w4_hbm, o_ref,
            kland, kres, vres, wqland, wqres, woland, wores, w3buf, w4buf, acc_ref,
            q_ref, s_ref, e_ref, inv_ref, lhs_ref, d_ref, x_ref,
            sem_k, sem_v, sem_q, sem_o, sem_w, *, sk):
    def k_copy(i):
        return pltpu.make_async_copy(
            k_hbm.at[pl.ds(i * _R, _R), pl.ds(sk - _W, _W)], kland.at[i % 2], sem_k.at[i % 2])

    def wq_copy(i):
        return pltpu.make_async_copy(
            wq_hbm.at[:, pl.ds(i * _R, _R)], wqland.at[i % 2], sem_q.at[i % 2])

    def wo_copy(i):
        return pltpu.make_async_copy(
            wo_hbm.at[pl.ds(i * _R, _R), :], woland.at[i % 2], sem_o.at[i % 2])

    def v_copy(i):
        return pltpu.make_async_copy(
            v_hbm.at[pl.ds(i * _R, _R), pl.ds(sk - _W, _W)],
            vres.at[pl.ds(i * _R, _R), :], sem_v.at[i % 3])

    def start_pair(i):
        wq_copy(i).start()
        k_copy(i).start()
        wo_copy(i).start()

    x_copy = pltpu.make_async_copy(x_hbm, x_ref, sem_w.at[0])
    w3_copy = pltpu.make_async_copy(w3_hbm, w3buf.at[:, pl.ds(0, _F)], sem_w.at[0])
    w4_copies = [
        pltpu.make_async_copy(w4_hbm.at[_W4[n]:_W4[n + 1], :], w4buf.at[_W4[n]:_W4[n + 1], :],
                              sem_w.at[1 + n])
        for n in range(_NW4)
    ]

    def mlp_hidden(x, c):
        y, c = _layernorm_near(x, c)
        yn = jnp.broadcast_to(_layernorm_near(y, 0.0)[0], (8, _D)).astype(_BF)
        return y, _gelu(_dot(yn, w3buf[:, 0:_F])).astype(_BF), c

    def mlp_out(x, y, h, wait):
        out = x + y
        for n in range(_NW4):
            if wait:
                w4_copies[n].wait()
            out = out + _dot(h[:, _W4[n]:_W4[n + 1]], w4buf[_W4[n]:_W4[n + 1], :])[0:1]
        return out

    start_pair(0)
    v_copy(0).start()
    x_copy.start()
    start_pair(1)
    v_copy(1).start()

    own, first = _pair_masks()
    x_copy.wait()
    x = x_ref[...].astype(_F32)
    always = ~(jnp.abs(jnp.broadcast_to(x[:, 0:128], (8, 128))) < 0.0)
    c = jnp.mean(x, axis=-1, keepdims=True)
    xn8 = jnp.broadcast_to(_layernorm(x), (8, _D)).astype(_BF)
    acc_ref[...] = jnp.zeros_like(acc_ref)

    @pl.loop(0, _NP)
    def _(i):
        wq_copy(i).wait()
        k_copy(i).wait()
        wo_copy(i).wait()
        v_copy(i).wait()

        @pl.when(i + 2 < _NP)
        def _():
            v_copy(i + 2).start()

        half = pl.multiple_of(i * _DH, _DH)
        full = pl.multiple_of(i * _R, _R)
        wq = wqland[i % 2]
        wo = woland[i % 2]
        wqres[:, pl.ds(full, _R)] = pltpu.bitcast(wq, _U32)
        wores[pl.ds(half, _DH), :] = pltpu.bitcast(wo, _U32)
        q = jnp.where(own, _dot(xn8, wq) * _C2, 0.0).astype(_BF)
        k = kland[i % 2]
        kres[pl.ds(half, _DH), :] = pltpu.bitcast(k, _U32)
        e, _, inv = _softmax_parts(_dot(q, k), first)
        o = _dot_t(e.astype(_BF), vres[pl.ds(full, _R), :])
        acc_ref[...] += _dot((jnp.where(own, o, 0.0) * inv).astype(_BF), wo)

        @pl.when(i + 2 < _NP)
        def _():
            start_pair(i + 2)

        @pl.when(i + 2 == _NP)
        def _():
            w3_copy.start()
            for w in w4_copies:
                w.start()

    x = x + jnp.sum(acc_ref[...], axis=0, keepdims=True)
    w3_copy.wait()
    y, h, c = mlp_hidden(x, c)
    x = mlp_out(x, y, h, wait=True)

    xn, c = _layernorm_near(x, c)
    xn8 = jnp.broadcast_to(xn, (8, _D)).astype(_BF)
    _layer2(xn8, always, kres, vres, wqres, wores,
            q_ref, s_ref, e_ref, inv_ref, lhs_ref, d_ref, acc_ref)
    x = x + jnp.sum(acc_ref[...], axis=0, keepdims=True)
    y, h, _ = mlp_hidden(x, c)
    o_ref[...] = mlp_out(x, y, h, wait=False).astype(o_ref.dtype)


@jax.jit
def pallas_interleave_layers__sliding_block_cached__mixer_s_mlp__decode_kernel(
    A_x: jax.Array,
    A_k_cache: jax.Array,
    A_v_cache: jax.Array,
    A_wq: jax.Array,
    A_wo: jax.Array,
    B_x: jax.Array,
    B_w1: jax.Array,
    B_w2: jax.Array,
    B_w3: jax.Array,
    B_w4: jax.Array,
):
    del B_x, B_w1, B_w2
    _, hkv, sk, dh = A_k_cache.shape
    assert A_x.shape == (1, 1, _D) and (hkv, dh) == (_H, _DH)
    assert min(4096, max(256, sk // 4)) == _W
    kt = jnp.swapaxes(A_k_cache, 2, 3).reshape(_H * _DH, sk)
    vt = jnp.swapaxes(A_v_cache, 2, 3).reshape(_H * _DH, sk)
    out = pl.pallas_call(
        functools.partial(_kernel, sk=sk),
        out_shape=jax.ShapeDtypeStruct((1, _D), A_x.dtype),
        in_specs=[pl.BlockSpec(memory_space=pl.ANY)] * 7,
        out_specs=pl.BlockSpec(memory_space=pltpu.VMEM),
        scratch_shapes=[
            pltpu.VMEM((2, _R, _W), _BF),
            pltpu.VMEM((_H * _DH // 2, _W), _U32),
            pltpu.VMEM((_H * _DH, _W), _BF),
            pltpu.VMEM((2, _D, _R), _BF),
            pltpu.VMEM((_D // 2, _H * _DH), _U32),
            pltpu.VMEM((2, _R, _D), _BF),
            pltpu.VMEM((_H * _DH // 2, _D), _U32),
            pltpu.VMEM((_D, _F + 128), _BF),
            pltpu.VMEM((_F, _D), _BF),
            pltpu.VMEM((8, _D), _F32),
            pltpu.VMEM((2, 8, _R), _F32),
            pltpu.VMEM((2, 8, _W), _F32),
            pltpu.VMEM((2, 8, _W), _F32),
            pltpu.VMEM((2, 8, _R), _F32),
            pltpu.VMEM((2, 8, _R), _F32),
            pltpu.VMEM((_RV + 64, 128), _F32),
            pltpu.VMEM((1, _D), _BF),
            pltpu.SemaphoreType.DMA((2,)),
            pltpu.SemaphoreType.DMA((3,)),
            pltpu.SemaphoreType.DMA((2,)),
            pltpu.SemaphoreType.DMA((2,)),
            pltpu.SemaphoreType.DMA((1 + _NW4,)),
        ],
        compiler_params=pltpu.CompilerParams(vmem_limit_bytes=127 * 1024 * 1024),
        name="interleave_decode",
    )(A_x.reshape(1, _D), kt, vt, A_wq, A_wo, B_w3, B_w4)
    return out.reshape(1, 1, _D)
```

```python
import functools

import jax
import jax.numpy as jnp
import jax.experimental.pallas as pl
import jax.experimental.pallas.tpu as pltpu
from jax import lax

_H = 32
_DH = 192
_W = 4096
_D = 640
_F = 1536
_EPS = 1e-5
_BF = jnp.bfloat16
_F32 = jnp.float32
_U32 = jnp.uint32

_NP = _H // 2
_R = 2 * _DH
_W4 = (0, 768, 1280, 1536)
_NW4 = len(_W4) - 1
_C2 = float(_DH) ** -0.5 * 1.4426950408889634

_CK = 512
_CX = 512
_RV = 32
_RX = _DH
_RAMP = 5
_T_W = 140.0
_T_QK = 96.0
_T_PX = _RX * _CX / 2048 * 2.05
_T_PV = _RV * _W / 2048 * 1.6
_T_STEP = _T_PV * _R / _RV
_T_MXU = 20.0
_T_START = 40.0
_T_MAX = 150.0
_T_SUM = 900.0
_T_SUM_RAMP = 450.0
_T_FOLD = 900.0


def _layernorm(x):
    m = jnp.mean(x, axis=-1, keepdims=True)
    d = x - m
    v = jnp.mean(d * d, axis=-1, keepdims=True)
    return d / jnp.sqrt(v + _EPS)


def _layernorm_near(x, c):
    d = x - c
    m = jnp.mean(d, axis=-1, keepdims=True)
    v = jnp.mean(d * d, axis=-1, keepdims=True) - m * m
    return (d - m) / jnp.sqrt(jnp.maximum(v, 0.0) + _EPS), c + m


def _gelu(x):
    c = 0.7978845608028654
    return 0.5 * x * (1.0 + jnp.tanh(c * (x + 0.044715 * (x * x * x))))


def _dot(a, b):
    return jnp.dot(a, b, preferred_element_type=_F32)


def _dot_t(a, b):
    return lax.dot_general(a, b, (((1,), (1,)), ((), ())), preferred_element_type=_F32)


def _pair_masks():
    row = lax.broadcasted_iota(jnp.int32, (8, _R), 0)
    col = lax.broadcasted_iota(jnp.int32, (8, _R), 1)
    own = (col >= row * _DH) & (col < (row + 1) * _DH)
    return own, col < _DH


def _softmax_parts(s, first):
    m = jnp.max(s, axis=-1, keepdims=True)
    e = jnp.exp2(s - m)
    inv = 1.0 / jnp.sum(e, axis=-1, keepdims=True)
    return e, m, jnp.where(first, inv[0:1, :], inv[1:2, :])


def _layer2(xn8, always, kres, vres, wqres, wores,
            q_ref, s_ref, e_ref, inv_ref, lhs_ref, d_ref, acc_ref):
    own, first = _pair_masks()
    sub = lax.broadcasted_iota(jnp.int32, (8, 128), 0)
    lane = lax.broadcasted_iota(jnp.int32, (8, 128), 1)
    nck = _W // _CK
    nrv = _DH // _RV

    def tie(a, b):
        return jnp.where(always, a, b)

    def span(start, n, align):
        return pl.ds(start if isinstance(start, int) else pl.multiple_of(start, align), n)

    def q_unit(i, slot):
        q8 = _dot(xn8, pltpu.bitcast(wqres[:, span(i * _R, _R, _R)], _BF))
        q_ref[slot] = jnp.where(own, q8 * _C2, 0.0)
        return q8[:, 0:128]

    def qk_unit(i, slot, c):
        cols = slice(c * _CK, (c + 1) * _CK)
        k = pltpu.bitcast(kres[span(i * _DH, _DH, _DH), cols], _BF)
        s = _dot(q_ref[slot].astype(_BF), k)
        s_ref[slot, :, cols] = s
        return s[:, 0:128]

    def o_unit(i, lhs):
        r = _dot(lhs.astype(_BF), pltpu.bitcast(wores[span(i * _DH, _DH, _DH), :], _BF))
        acc_ref[...] += r
        return r[:, 0:128]

    def px_unit(i, slot, c, ox):
        cols = slice(c * _CX, (c + 1) * _CX)
        o = _dot_t(e_ref[slot, :, cols].astype(_BF), vres[pl.ds((i + 1) * _R - _RX, _RX), cols])
        ox[0] = o if c == 0 else ox[0] + o
        return jnp.broadcast_to(o[:, 0:1], (8, 128))

    def softmax(slot):
        e, m, inv = _softmax_parts(s_ref[slot], first)
        e_ref[slot] = e
        inv_ref[slot] = inv
        return jnp.broadcast_to(m, (8, 128)), inv[:, 0:128]

    def fold(a, red):
        a = jnp.broadcast_to(jnp.sum(a, axis=1, keepdims=True), a.shape)
        for b in range(a.shape[0] // 8):
            v, w = a[8 * b:8 * b + 8], 8
            while red and red[-1][0] == w and w < 128:
                v = jnp.where((lane & w) == 0, red.pop()[1], v)
                w *= 2
            red.append((w, v))
        return red[-1][1]

    def pv_unit(i, slot, hh, c, ties, red, park):
        rows = span(i * _R + hh * _DH + c * _RV, _RV, _RV)
        a = None
        for t in ties:
            a = tie(jnp.zeros((8, 128), _F32) if a is None else a, t)
        if a is not None:
            a = jnp.tile(a, (_RV // 8, 1))
        accs = [a, None]
        for j in range(_W // 128):
            cols = slice(j * 128, (j + 1) * 128)
            p = jnp.broadcast_to(e_ref[slot, hh:hh + 1, cols], (8, 128))
            t = vres[rows, cols].astype(_F32) * jnp.tile(p, (_RV // 8, 1))
            n = j // 2 % 2
            accs[n] = t if accs[n] is None else accs[n] + t
        a = accs[0] + accs[1]
        if park:
            d_ref[0:_RV, :] = a
            return a[0:8]
        return fold(a, red)

    def make_lhs(slot, red, ox=None):
        parts = [jnp.where((lane & 7) == sub, v, 0.0)[:, 0:w] for (w, v) in red]
        if ox is not None:
            parts.append(jnp.where(own[:, _R - _RX:], ox[0], 0.0))
        return jnp.concatenate(parts, axis=1) * inv_ref[slot]

    def unpark(slot):
        widths = []
        for _ in range((_R - _RV) // 8):
            w = 8
            while widths and widths[-1] == w and w < 128:
                widths.pop()
                w *= 2
            widths.append(w)
        red = [(w, d_ref[_RV + 8 * n:_RV + 8 * n + 8, :]) for n, w in enumerate(widths)]
        fold(d_ref[0:_RV, :], red)
        return make_lhs(slot, red)

    def step(i, par, mxu, carry, *, sm_after=0, sm=True, out=True, parked=True, park=True, px=False):
        mxu = list(mxu)
        if out:
            lhs = unpark(1 - par) if parked else None
            mxu.append((_T_W, lambda: o_unit(i - 1, lhs_ref[1 - par] if lhs is None else lhs)))
        ox = [None]
        if px:
            mxu = [(_T_PX, functools.partial(px_unit, i, par, c, ox)) for c in range(_W // _CX)] + mxu
        mxu.reverse()
        pending = [(t - _T_STEP, v) for (t, v) in carry]
        if sm and sm_after == 0:
            pending += zip((_T_MAX, _T_SUM), softmax(1 - par))
        tm, done = 0.0, 0

        def run_mxu():
            nonlocal tm, done
            dt, fn = mxu.pop()
            tm += dt
            done += 1
            pending.append((tm + _T_MXU, fn()))
            if sm and done == sm_after:
                pending.extend(zip((tm + _T_MAX, tm + _T_SUM_RAMP), softmax(1 - par)))

        tv, red = _T_START, []
        for hh in range(2):
            for c in range(0 if px and hh else nrv):
                while mxu and tm + _T_MXU <= tv + 2 * _T_PV + 200:
                    run_mxu()
                ties = [v for (t, v) in pending if t <= tv]
                pending[:] = [(t, v) for (t, v) in pending if t > tv]
                v = pv_unit(i, par, hh, c, ties, red, park and hh == 1 and c == nrv - 1)
                tv += _T_PV
                pending.append((tv + _T_FOLD, v))
        while mxu:
            run_mxu()
        if park:
            for n, (_, v) in enumerate(red):
                d_ref[_RV + 8 * n:_RV + 8 * n + 8, :] = v
        else:
            lhs_ref[par] = make_lhs(par, red, ox if px else None)
        return pending

    def q(i, par):
        return [(_T_W, functools.partial(q_unit, i, par))]

    def qk(i, par, lo=0, hi=nck):
        return [(_T_QK, functools.partial(qk_unit, i, par, c)) for c in range(lo, hi)]

    acc_ref[...] = jnp.zeros_like(acc_ref)
    for _, fn in q(0, 0) + q(1, 1) + qk(0, 0):
        fn()
    softmax(0)
    carry = step(0, 0, qk(1, 1) + q(2, 0) + qk(2, 0, 0, _RAMP), (),
                 sm_after=nck, out=False)
    carry = step(1, 1, qk(2, 0, _RAMP) + q(3, 1) + qk(3, 1) + q(4, 0), carry,
                 sm_after=nck - _RAMP)
    carry = step(2, 0, qk(4, 0) + q(5, 1), carry)

    @pl.loop(0, (_NP - 6) // 2)
    def _(n):
        carry = ()
        for u in (3, 4):
            i, par = 2 * n + u, u % 2
            carry = step(i, par, qk(i + 2, par) + q(i + 3, 1 - par), carry)

    n = _NP - 3
    carry = step(n, 1, qk(n + 2, 1), (), park=False)
    carry = step(n + 1, 0, [], carry, parked=False, park=False, px=True)
    carry = step(n + 2, 1, [], carry, parked=False, park=False, px=True, sm=False)
    o_unit(n + 2, lhs_ref[1])


def _kernel(x_hbm, k_hbm, v_hbm, wq_hbm, wo_hbm, w3_hbm, w4_hbm, o_ref,
            kland, kres, vres, wqland, wqres, woland, wores, w3buf, w4buf, acc_ref,
            q_ref, s_ref, e_ref, inv_ref, lhs_ref, d_ref, x_ref,
            sem_k, sem_v, sem_q, sem_o, sem_w, *, sk):
    def k_copy(i):
        return pltpu.make_async_copy(
            k_hbm.at[pl.ds(i * _R, _R), pl.ds(sk - _W, _W)], kland.at[i % 2], sem_k.at[i % 2])

    def wq_copy(i):
        return pltpu.make_async_copy(
            wq_hbm.at[:, pl.ds(i * _R, _R)], wqland.at[i % 2], sem_q.at[i % 2])

    def wo_copy(i):
        return pltpu.make_async_copy(
            wo_hbm.at[pl.ds(i * _R, _R), :], woland.at[i % 2], sem_o.at[i % 2])

    def v_copy(i):
        return pltpu.make_async_copy(
            v_hbm.at[pl.ds(i * _R, _R), pl.ds(sk - _W, _W)],
            vres.at[pl.ds(i * _R, _R), :], sem_v.at[i % 3])

    def start_pair(i):
        wq_copy(i).start()
        k_copy(i).start()
        wo_copy(i).start()

    x_copy = pltpu.make_async_copy(x_hbm, x_ref, sem_w.at[0])
    w3_copy = pltpu.make_async_copy(w3_hbm, w3buf.at[:, pl.ds(0, _F)], sem_w.at[0])
    w4_copies = [
        pltpu.make_async_copy(w4_hbm.at[_W4[n]:_W4[n + 1], :], w4buf.at[_W4[n]:_W4[n + 1], :],
                              sem_w.at[1 + n])
        for n in range(_NW4)
    ]

    def mlp_hidden(x, c):
        y, c = _layernorm_near(x, c)
        yn = jnp.broadcast_to(_layernorm_near(y, 0.0)[0], (8, _D)).astype(_BF)
        return y, _gelu(_dot(yn, w3buf[:, 0:_F])).astype(_BF), c

    def mlp_out(x, y, h, wait):
        out = x + y
        for n in range(_NW4):
            if wait:
                w4_copies[n].wait()
            out = out + _dot(h[:, _W4[n]:_W4[n + 1]], w4buf[_W4[n]:_W4[n + 1], :])[0:1]
        return out

    start_pair(0)
    v_copy(0).start()
    x_copy.start()
    start_pair(1)
    v_copy(1).start()

    own, first = _pair_masks()
    x_copy.wait()
    x = x_ref[...].astype(_F32)
    always = ~(jnp.abs(jnp.broadcast_to(x[:, 0:128], (8, 128))) < 0.0)
    c = jnp.mean(x, axis=-1, keepdims=True)
    xn8 = jnp.broadcast_to(_layernorm(x), (8, _D)).astype(_BF)
    acc_ref[...] = jnp.zeros_like(acc_ref)

    @pl.loop(0, _NP)
    def _(i):
        wq_copy(i).wait()
        k_copy(i).wait()
        wo_copy(i).wait()
        v_copy(i).wait()

        @pl.when(i + 2 < _NP)
        def _():
            v_copy(i + 2).start()

        half = pl.multiple_of(i * _DH, _DH)
        full = pl.multiple_of(i * _R, _R)
        wq = wqland[i % 2]
        wo = woland[i % 2]
        wqres[:, pl.ds(full, _R)] = pltpu.bitcast(wq, _U32)
        wores[pl.ds(half, _DH), :] = pltpu.bitcast(wo, _U32)
        q = jnp.where(own, _dot(xn8, wq) * _C2, 0.0).astype(_BF)
        k = kland[i % 2]
        kres[pl.ds(half, _DH), :] = pltpu.bitcast(k, _U32)
        e, _, inv = _softmax_parts(_dot(q, k), first)
        o = _dot_t(e.astype(_BF), vres[pl.ds(full, _R), :])
        acc_ref[...] += _dot((jnp.where(own, o, 0.0) * inv).astype(_BF), wo)

        @pl.when(i + 2 < _NP)
        def _():
            start_pair(i + 2)

        @pl.when(i + 2 == _NP)
        def _():
            w3_copy.start()
            for w in w4_copies:
                w.start()

    x = x + jnp.sum(acc_ref[...], axis=0, keepdims=True)
    w3_copy.wait()
    y, h, c = mlp_hidden(x, c)
    x = mlp_out(x, y, h, wait=True)

    xn, c = _layernorm_near(x, c)
    xn8 = jnp.broadcast_to(xn, (8, _D)).astype(_BF)
    _layer2(xn8, always, kres, vres, wqres, wores,
            q_ref, s_ref, e_ref, inv_ref, lhs_ref, d_ref, acc_ref)
    x = x + jnp.sum(acc_ref[...], axis=0, keepdims=True)
    y, h, _ = mlp_hidden(x, c)
    o_ref[...] = mlp_out(x, y, h, wait=False).astype(o_ref.dtype)


@jax.jit
def pallas_interleave_layers__sliding_block_cached__mixer_s_mlp__decode_kernel(
    A_x: jax.Array,
    A_k_cache: jax.Array,
    A_v_cache: jax.Array,
    A_wq: jax.Array,
    A_wo: jax.Array,
    B_x: jax.Array,
    B_w1: jax.Array,
    B_w2: jax.Array,
    B_w3: jax.Array,
    B_w4: jax.Array,
):
    del B_x, B_w1, B_w2
    _, hkv, sk, dh = A_k_cache.shape
    assert A_x.shape == (1, 1, _D) and (hkv, dh) == (_H, _DH)
    assert min(4096, max(256, sk // 4)) == _W
    kt = jnp.swapaxes(A_k_cache, 2, 3).reshape(_H * _DH, sk)
    vt = jnp.swapaxes(A_v_cache, 2, 3).reshape(_H * _DH, sk)
    out = pl.pallas_call(
        functools.partial(_kernel, sk=sk),
        out_shape=jax.ShapeDtypeStruct((1, _D), A_x.dtype),
        in_specs=[pl.BlockSpec(memory_space=pl.ANY)] * 7,
        out_specs=pl.BlockSpec(memory_space=pltpu.VMEM),
        scratch_shapes=[
            pltpu.VMEM((2, _R, _W), _BF),
            pltpu.VMEM((_H * _DH // 2, _W), _U32),
            pltpu.VMEM((_H * _DH, _W), _BF),
            pltpu.VMEM((2, _D, _R), _BF),
            pltpu.VMEM((_D // 2, _H * _DH), _U32),
            pltpu.VMEM((2, _R, _D), _BF),
            pltpu.VMEM((_H * _DH // 2, _D), _U32),
            pltpu.VMEM((_D, _F + 128), _BF),
            pltpu.VMEM((_F, _D), _BF),
            pltpu.VMEM((8, _D), _F32),
            pltpu.VMEM((2, 8, _R), _F32),
            pltpu.VMEM((2, 8, _W), _F32),
            pltpu.VMEM((2, 8, _W), _F32),
            pltpu.VMEM((2, 8, _R), _F32),
            pltpu.VMEM((2, 8, _R), _F32),
            pltpu.VMEM((_RV + 64, 128), _F32),
            pltpu.VMEM((1, _D), _BF),
            pltpu.SemaphoreType.DMA((2,)),
            pltpu.SemaphoreType.DMA((3,)),
            pltpu.SemaphoreType.DMA((2,)),
            pltpu.SemaphoreType.DMA((2,)),
            pltpu.SemaphoreType.DMA((1 + _NW4,)),
        ],
        compiler_params=pltpu.CompilerParams(vmem_limit_bytes=127 * 1024 * 1024),
        name="interleave_decode",
    )(A_x.reshape(1, _D), kt, vt, A_wq, A_wo, B_w3, B_w4)
    return out.reshape(1, 1, _D)
```
